```python
import jax
import jax.numpy as jnp

def _softmax(x, axis=-1):
    return jax.nn.softmax(x, axis=axis)

def _gelu(x):
    return jax.nn.gelu(x, approximate=True)

def _silu(x):
    return jax.nn.silu(x)

def _sigmoid(x):
    return jax.nn.sigmoid(x)

def _layernorm(x, axis=-1, eps=1e-05):
    m = jnp.mean(x, axis=axis, keepdims=True)
    v = jnp.var(x, axis=axis, keepdims=True)
    return (x - m) / jnp.sqrt(v + eps)

def _scatter_add(tgt, idx, src, axis=0):
    return tgt.at[idx].add(src)

def _segment_sum(src, seg, n):
    return jax.ops.segment_sum(src, seg, n)

class _Rng:

    def __init__(self, key):
        self._k = key

    def _next(self):
        self._k, sub = jax.random.split(self._k)
        return sub

    def normal(self, shape):
        return jax.random.normal(self._next(), shape, dtype=jnp.bfloat16)

    def randint(self, lo, hi, shape):
        return jax.random.randint(self._next(), shape, lo, hi, dtype=jnp.int32)

    def uniform(self, shape, lo=0.0, hi=1.0):
        return jax.random.uniform(self._next(), shape, jnp.bfloat16, lo, hi)

    def permutation(self, n):
        return jax.random.permutation(self._next(), n)
kernel_name = 'interleave_layers__memory_aug_infini_attn__mixer_s_mlp__prompt'

def setup_inputs():
    _rng = _Rng(jax.random.key(int.from_bytes(__import__("os").urandom(4), "little")))
    _w = lambda a: (lambda t: t.astype(jnp.bfloat16) if jnp.issubdtype(t.dtype, jnp.floating) else t)(jnp.asarray(a))

    def _A_setup():
        B, S, D, H = (1, 2048, 1024, 32)
        N = 4
        L = max(1, S // N)
        sc = D ** (-0.5)
        return {'x': _w((lambda *s: _rng.normal(s) * 0.05)(B, N * L, D)), 'wq': _w((lambda *s: _rng.normal(s) * 0.05)(D, D) * sc), 'wk': _w((lambda *s: _rng.normal(s) * 0.05)(D, D) * sc), 'wv': _w((lambda *s: _rng.normal(s) * 0.05)(D, D) * sc), 'wo': _w((lambda *s: _rng.normal(s) * 0.05)(D, D) * sc), 'beta': _w((lambda *s: _rng.normal(s) * 0.05)(H))}
    _A_in = _A_setup()

    def _B_setup():
        B, S, D, F = (1, 2048, 1024, 3584)
        return {'x': _w((lambda *s: _rng.normal(s) * 0.05)(B, S, D)), 'w1': _w((lambda *s: _rng.normal(s) * 0.05)(D, D) * D ** (-0.5)), 'w2': _w((lambda *s: _rng.normal(s) * 0.05)(D, D) * D ** (-0.5)), 'w3': _w((lambda *s: _rng.normal(s) * 0.05)(D, F) * D ** (-0.5)), 'w4': _w((lambda *s: _rng.normal(s) * 0.05)(F, D) * F ** (-0.5))}
    _B_in = _B_setup()
    return {'A_x': _A_in['x'], 'A_wq': _A_in['wq'], 'A_wk': _A_in['wk'], 'A_wv': _A_in['wv'], 'A_wo': _A_in['wo'], 'A_beta': _A_in['beta'], 'B_x': _B_in['x'], 'B_w1': _B_in['w1'], 'B_w2': _B_in['w2'], 'B_w3': _B_in['w3'], 'B_w4': _B_in['w4']}

def reference(A_x, A_wq, A_wk, A_wv, A_wo, A_beta, B_x, B_w1, B_w2, B_w3, B_w4):

    def _A_ref(x, wq, wk, wv, wo, beta):
        B, S, D = x.shape
        H = 32
        Dh = D // H
        N = 4
        L = S // N
        q = (lambda x, *d: x.transpose(*d))((x @ wq).reshape(B, S, H, Dh), 0, 2, 1, 3).reshape(B, H, N, L, Dh)
        k = (lambda x, *d: x.transpose(*d))((x @ wk).reshape(B, S, H, Dh), 0, 2, 1, 3).reshape(B, H, N, L, Dh)
        v = (lambda x, *d: x.transpose(*d))((x @ wv).reshape(B, S, H, Dh), 0, 2, 1, 3).reshape(B, H, N, L, Dh)
        phi = lambda t: jnp.where(t > 0, t + 1.0, jnp.exp(t))
        scale = Dh ** (-0.5)
        ar = jnp.arange(L)
        mask = (lambda x, dt: x.astype(dt))(ar[:, None] < ar[None, :], x.dtype) * -1000000000.0
        g = _sigmoid(beta).reshape(1, H, 1, 1)
        M = jnp.einsum('bhd,bhe->bhde', q[:, :, 0, 0, :] * 0.0, q[:, :, 0, 0, :] * 0.0)
        z = q[:, :, 0, 0, :] * 0.0
        outs = []
        for s in range(N):
            qs, ks, vs = (q[:, :, s].copy(), k[:, :, s].copy(), v[:, :, s].copy())
            logits = jnp.einsum('bhqd,bhkd->bhqk', qs, ks) * scale + mask
            p = _softmax(logits, axis=-1)
            a_dot = jnp.einsum('bhqk,bhkd->bhqd', p, vs)
            pq = phi(qs)
            num = jnp.einsum('bhld,bhde->bhle', pq, M)
            den = jnp.einsum('bhld,bhd->bhl', pq, z)[..., None] + 1e-06
            a_mem = num / den
            o = g * a_mem + (1.0 - g) * a_dot
            outs.append(o)
            pk = phi(ks)
            M = M + jnp.einsum('bhld,bhle->bhde', pk, vs)
            z = z + jnp.einsum('bhld->bhd', pk)
        o = (lambda x, *d: x.transpose(*d))(jnp.stack(outs, 2).reshape(B, H, S, Dh), 0, 2, 1, 3).reshape(B, S, D)
        return o @ wo

    def _B_ref(x, w1, w2, w3, w4):
        B, S, D = x.shape
        h = _gelu(_layernorm(x, axis=-1) @ w1)
        c = D // 4
        g0 = jnp.pad(h[:, :, 0 * c:1 * c], ((0, 0), (1, 0), (0, 0)))[:, :S, :]
        g1 = jnp.pad(h[:, :, 1 * c:2 * c], ((0, 0), (0, 1), (0, 0)))[:, 1:, :]
        g2 = jnp.pad(h[:, :, 2 * c:3 * c], ((0, 0), (2, 0), (0, 0)))[:, :S, :]
        g3 = jnp.pad(h[:, :, 3 * c:], ((0, 0), (0, 2), (0, 0)))[:, 2:, :]
        hs = jnp.concatenate([g0, g1, g2, g3], axis=-1) @ w2
        x1 = x + hs
        h2 = _gelu(_layernorm(x1, axis=-1) @ w3) @ w4
        return x1 + h2
    x = A_x
    x = x + _A_ref(_layernorm(x, axis=-1), A_wq, A_wk, A_wv, A_wo, A_beta)
    x = x + _B_ref(_layernorm(x, axis=-1), B_w1, B_w2, B_w3, B_w4)
    x = x + _A_ref(_layernorm(x, axis=-1), A_wq, A_wk, A_wv, A_wo, A_beta)
    x = x + _B_ref(_layernorm(x, axis=-1), B_w1, B_w2, B_w3, B_w4)
    return x
```

```python
import functools

import jax
import jax.numpy as jnp
from jax import lax
import jax.experimental.pallas as pl
import jax.experimental.pallas.tpu as pltpu

S = 2048
D = 1024
H = 32
DH = 32
NSEG = 4
L = S // NSEG
F = 3584
NG = D // 128
HPG = 128 // DH
NT = L // 128
EPS = 1e-5
LOG2E = 1.4426950408889634
QSCALE = (DH ** -0.5) * LOG2E
NEG = -1e30
PADR = 8
MROWS = 144

import os
DEPTH = int(os.environ.get('DEPTH', '2'))
STAGE = int(os.environ.get('STAGE', '0'))
NATT = int(os.environ.get('NATT', '8'))
REPB = int(os.environ.get('REPB', '1'))
REPA = int(os.environ.get('REPA', '1'))
NLAY = int(os.environ.get('NLAY', '2'))
F32 = jnp.float32
BF16 = jnp.bfloat16
U32 = jnp.uint32


def _dot(a, b):
    return jnp.dot(a, b, preferred_element_type=F32)


def _dot_nt(a, b):
    return lax.dot_general(a, b, (((1,), (1,)), ((), ())), preferred_element_type=F32)


def _dot_tn(a, b):
    return lax.dot_general(a, b, (((0,), (0,)), ((), ())), preferred_element_type=F32)


def _layernorm(x):
    m = jnp.mean(x, axis=-1, keepdims=True)
    xc = x - m
    v = jnp.mean(xc * xc, axis=-1, keepdims=True)
    return xc * lax.rsqrt(v + EPS)


def _gelu(x):
    c = 0.7978845608028654
    inner = x * (c + (c * 0.044715) * (x * x))
    hx = 0.5 * x
    return hx + hx * jnp.tanh(inner)


def _pack(x):
    return pltpu.bitcast(x.astype(BF16), U32)


def _unpack(x):
    return pltpu.bitcast(x, BF16)


def _recip(x):
    r = pl.reciprocal(x, approx=True)
    return r * (2.0 - x * r)


def _phi(t):
    return jnp.where(t > 0, t + 1.0, jnp.exp(t))


def _kernel(x_hbm, wq_hbm, wk_hbm, wv_hbm, wo_hbm, beta_ref, w1_hbm, w2_hbm, w3_hbm, w4_hbm,
            out_hbm,
            xb, xa, ybuf, hbuf, wq, wk, wv, wvt, wo, w1, w2, w3, w4,
            qs, pq, kk, pk, vt, ot, mt, zb, gb, sbuf, in_sems, out_sems):

    def x_copy(s):
        return pltpu.make_async_copy(x_hbm.at[0, pl.ds(s * L, L), :], xb.at[pl.ds(s * L, L), :],
                                     in_sems.at[s])

    def out_copy(s):
        return pltpu.make_async_copy(xb.at[pl.ds(s * L, L), :], out_hbm.at[0, pl.ds(s * L, L), :],
                                     out_sems.at[s])

    w_copies = [pltpu.make_async_copy(src, dst, in_sems.at[NSEG + i])
                for i, (src, dst) in enumerate([(wq_hbm, wq), (wk_hbm, wk), (wv_hbm, wv), (wo_hbm, wo),
                                                (w1_hbm, w1), (w2_hbm, w2), (w3_hbm, w3), (w4_hbm, w4)])]

    w_copies[2].start()
    x_copy(0).start()
    w_copies[0].start()
    w_copies[1].start()

    beta = beta_ref[...].astype(F32)
    g_row = 1.0 / (1.0 + jnp.exp(-beta))
    eye = lax.broadcasted_iota(jnp.int32, (H, H), 0) == lax.broadcasted_iota(jnp.int32, (H, H), 1)
    g_col = jnp.sum(jnp.where(eye, g_row, 0.0), axis=1, keepdims=True)
    gb[...] = jnp.broadcast_to(g_col, (H, 128))

    zero_pad = jnp.zeros((NG, PADR, 128), F32)
    hbuf[:, 0:PADR, :] = zero_pad
    hbuf[:, PADR + S:PADR + S + PADR, :] = zero_pad

    w_copies[2].wait()
    wvt[...] = wv[...].T

    def attn_group(g, s):
        lane = lax.broadcasted_iota(jnp.int32, (64, 128), 1)
        key_i = lax.broadcasted_iota(jnp.int32, (128, 128), 0)
        qry_i = lax.broadcasted_iota(jnp.int32, (128, 128), 1)
        causal = key_i <= qry_i
        causal4 = jnp.concatenate([causal] * HPG, axis=1)
        gates = [gb[pl.ds(g * HPG + h, 1), :] for h in range(HPG)]

        def qcat(j):
            qj = qs[g, j * 64:(j + 1) * 64, :]
            qc = jnp.concatenate(
                [jnp.where((lane >= h * DH) & (lane < (h + 1) * DH), qj, jnp.uint32(0))
                 for h in range(HPG)], axis=0)
            return pltpu.bitcast(qc, BF16)

        def scores(j, t, qc):
            st = _dot_nt(_unpack(kk[g, t * 64:(t + 1) * 64, :]), qc)
            if t == j:
                st = jnp.where(causal4, st, NEG)
            m = jnp.max(st, axis=0, keepdims=True)
            if STAGE:
                u = j * (j + 1) // 2 + t
                sbuf[u] = st
                st = jnp.concatenate([sbuf[u, :, h * 128:(h + 1) * 128] for h in range(HPG)], axis=1)
            p = jnp.exp2(st - m)
            l = jnp.sum(p.reshape(16, 8, HPG * 128), axis=0)
            return [p[:, h * 128:(h + 1) * 128].astype(BF16) for h in range(HPG)], m, l

        def pv_tile(t, p):
            return [_dot(_unpack(vt[g, h * 16:(h + 1) * 16, t * 128:(t + 1) * 128]), p[h])
                    for h in range(HPG)]

        def finish(j, parts, mem):
            m = parts[0][0]
            for mt_, _, _ in parts[1:]:
                m = jnp.maximum(m, mt_)
            if len(parts) > 1:
                alphas = [jnp.exp2(mt_ - m) for mt_, _, _ in parts]
                lp = sum(al * lt for al, (_, lt, _) in zip(alphas, parts))
            else:
                lp = parts[0][1]
            rl = _recip(jnp.sum(lp, axis=0, keepdims=True))
            rden = _recip(mem[128:136, j * 128:(j + 1) * 128] + 1e-6)
            for h in range(HPG):
                cs = slice(h * 128, (h + 1) * 128)
                r2 = (1.0 - gates[h]) * rl[:, cs]
                num = mem[h * DH:(h + 1) * DH, j * 128:(j + 1) * 128]
                o = num * (gates[h] * rden[h:h + 1])
                if len(parts) > 1:
                    for al, (_, _, pvs) in zip(alphas, parts):
                        o = o + pvs[h] * (al[:, cs] * r2)
                else:
                    o = o + parts[0][2][h] * r2
                ot[g, h * 16:(h + 1) * 16, j * 128:(j + 1) * 128] = _pack(o)

        mem = _dot_nt(mt[g].astype(BF16), _unpack(pq[g]))
        units = [(j, t) for j in reversed(range(NT)) for t in range(j + 1)]
        qcs = {}
        parts = {j: [] for j in range(NT)}
        pending = []

        def drain_one():
            j, t, p, m, l = pending.pop(0)
            parts[j].append((m, l, pv_tile(t, p)))
            if len(parts[j]) == j + 1:
                finish(j, parts[j], mem)

        for (j, t) in units:
            if j not in qcs:
                qcs[j] = qcat(j)
            pending.append((j, t) + scores(j, t, qcs[j]))
            if len(pending) > DEPTH:
                drain_one()
        upd = _dot(_unpack(vt[g]), _unpack(pk[g]))
        while pending:
            drain_one()
        bd = (key_i // DH) == (qry_i // DH)
        mt[g, 0:128, :] = mt[g, 0:128, :] + jnp.where(bd, upd, 0.0)
        zrow = lax.broadcasted_iota(jnp.int32, (MROWS - 128, 128), 0)
        zlane = lax.broadcasted_iota(jnp.int32, (MROWS - 128, 128), 1)
        mt[g, 128:MROWS, :] = mt[g, 128:MROWS, :] + jnp.where(zrow == zlane // DH, zb[g], 0.0)

    def phase_a(layer, s):
        layer = jnp.where(s < NSEG, layer, 5)
        s = s % NSEG
        r0 = pl.multiple_of(s * L, L)
        first = layer == 2 - NLAY

        @pl.when(first)
        def _():
            x_copy(s).wait()

        @pl.when(jnp.logical_and(first, s == 0))
        def _():
            w_copies[0].wait()
            w_copies[1].wait()
            w_copies[3].start()
            w_copies[4].start()
            for s2 in range(1, NSEG):
                x_copy(s2).start()

        @pl.when(s == 0)
        def _():
            mt[...] = jnp.zeros(mt.shape, F32)

        x = xb[pl.ds(r0, L), :].astype(F32)
        xn = _layernorm(x).astype(BF16)
        q = _dot(xn, wq[...])
        k = _dot(xn, wk[...])
        vtv = _dot_nt(wvt[...], xn)
        for g in range(NG):
            sl = slice(g * 128, (g + 1) * 128)
            qs[g] = _pack(q[:, sl] * QSCALE)
            pq[g] = _pack(_phi(q[:, sl]))
            kk[g] = _pack(k[:, sl])
            pkf = _phi(k[:, sl])
            pk[g] = _pack(pkf)
            zb[g] = jnp.sum(pkf, axis=0, keepdims=True)
            vt[g] = _pack(vtv[sl, :])

        def body(g, c):
            attn_group(g, s)
            return c
        lax.fori_loop(0, NATT, body, 0)

        @pl.when(jnp.logical_and(first, s == 0))
        def _():
            w_copies[3].wait()
            w_copies[4].wait()
            for c in w_copies[5:]:
                c.start()

        o_t = _unpack(ot[...].reshape(D // 2, L))
        x2 = xb[pl.ds(r0, L), :].astype(F32) + _dot_tn(o_t, wo[...])
        y = _layernorm(x2)
        xa[pl.ds(r0, L), :] = x2
        ybuf[pl.ds(r0, L), :] = y
        hv = _gelu(_dot(_layernorm(y).astype(BF16), w1[...]))
        hview = hbuf.at[:, pl.ds(r0, L + 2 * PADR), :]
        for g in range(NG):
            hview[g, PADR:PADR + L, :] = hv[:, g * 128:(g + 1) * 128]

    def phase_b(layer, s):
        layer = jnp.where(s < NSEG, layer, 5)
        s = s % NSEG
        r0 = pl.multiple_of(s * L, L)

        @pl.when(jnp.logical_and(layer == 2 - NLAY, s == 0))
        def _():
            w_copies[5].wait()
            w_copies[6].wait()
            w_copies[7].wait()

        hview = hbuf.at[:, pl.ds(r0, L + 2 * PADR), :]
        shifts = (-1, -1, 1, 1, -2, -2, 2, 2)
        hs_in = jnp.concatenate(
            [hview[g, PADR + shifts[g]:PADR + shifts[g] + L, :].astype(BF16) for g in range(NG)], axis=1)
        x1 = ybuf[pl.ds(r0, L), :] + _dot(hs_in, w2[...])
        t = xa[pl.ds(r0, L), :] + x1
        xn2 = _layernorm(x1).astype(BF16)
        h2 = _gelu(_dot(xn2, w3[...])).astype(BF16)
        res = t + _dot(h2, w4[...])
        xb[pl.ds(r0, L), :] = res.astype(BF16)

        @pl.when(layer == 1)
        def _():
            out_copy(s).start()

    def layer_body(layer, c):
        lax.fori_loop(0, NSEG * REPA, lambda s, c: (phase_a(layer, s), c)[1], 0)
        lax.fori_loop(0, NSEG * REPB, lambda s, c: (phase_b(layer, s), c)[1], 0)
        return c
    lax.fori_loop(2 - NLAY, 2, layer_body, 0)

    for s in range(NSEG):
        out_copy(s).wait()


@jax.jit
def pallas_interleave_layers__memory_aug_infini_attn__mixer_s_mlp__prompt_kernel(
    A_x: jax.Array,
    A_wq: jax.Array,
    A_wk: jax.Array,
    A_wv: jax.Array,
    A_wo: jax.Array,
    A_beta: jax.Array,
    B_x: jax.Array,
    B_w1: jax.Array,
    B_w2: jax.Array,
    B_w3: jax.Array,
    B_w4: jax.Array,
):
    del B_x
    hbm = pl.BlockSpec(memory_space=pl.ANY)
    vmem = pl.BlockSpec(memory_space=pltpu.VMEM)
    scratch = [
        pltpu.VMEM((S, D), BF16),
        pltpu.VMEM((S, D), F32),
        pltpu.VMEM((S, D), F32),
        pltpu.VMEM((NG, S + 2 * PADR, 128), F32),
        pltpu.VMEM((D, D), BF16),
        pltpu.VMEM((D, D), BF16),
        pltpu.VMEM((D, D), BF16),
        pltpu.VMEM((D, D), BF16),
        pltpu.VMEM((D, D), BF16),
        pltpu.VMEM((D, D), BF16),
        pltpu.VMEM((D, D), BF16),
        pltpu.VMEM((D, F), BF16),
        pltpu.VMEM((F, D), BF16),
        pltpu.VMEM((NG, L // 2, 128), U32),
        pltpu.VMEM((NG, L // 2, 128), U32),
        pltpu.VMEM((NG, L // 2, 128), U32),
        pltpu.VMEM((NG, L // 2, 128), U32),
        pltpu.VMEM((NG, 64, L), U32),
        pltpu.VMEM((NG, 64, L), U32),
        pltpu.VMEM((NG, MROWS, 128), F32),
        pltpu.VMEM((NG, 1, 128), F32),
        pltpu.VMEM((H, 128), F32),
        pltpu.VMEM((10, 128, 512), F32),
        pltpu.SemaphoreType.DMA((NSEG + 8,)),
        pltpu.SemaphoreType.DMA((NSEG,)),
    ]
    return pl.pallas_call(
        _kernel,
        out_shape=jax.ShapeDtypeStruct(A_x.shape, A_x.dtype),
        in_specs=[hbm, hbm, hbm, hbm, hbm, vmem, hbm, hbm, hbm, hbm],
        out_specs=hbm,
        scratch_shapes=scratch,
        compiler_params=pltpu.CompilerParams(vmem_limit_bytes=120 * 1024 * 1024),
    )(A_x, A_wq, A_wk, A_wv, A_wo, A_beta.reshape(1, H), B_w1, B_w2, B_w3, B_w4)
```

```python
from functools import partial, reduce

import jax
import jax.numpy as jnp
from jax import lax
import jax.experimental.pallas as pl
import jax.experimental.pallas.tpu as pltpu

S = 2048
D = 1024
H = 32
DH = 32
NSEG = 4
NLAYER = 2
NSTEP = NSEG * NLAYER
L = S // NSEG
F = 3584
NG = D // 128
HPG = 128 // DH
NT = L // 128
EPS = 1e-5
LOG2E = 1.4426950408889634
QSCALE = (DH ** -0.5) * LOG2E
NEG = -1e30
PADR = 8
MROWS = 144
MB = 256

SUBA = 4
SUBB = 2
W3A = 512
AORD = 'n0,n1,n2,n3,o0,o1,u0,o2,u1,o3,u2,u3'
RATE = 0.97
DELAY = 350
PVD = 32
CLEAD = 192
F32 = jnp.float32
BF16 = jnp.bfloat16
U32 = jnp.uint32


def _dot(a, b):
    return jnp.dot(a, b, preferred_element_type=F32)


def _dot_nt(a, b):
    return lax.dot_general(a, b, (((1,), (1,)), ((), ())), preferred_element_type=F32)


def _layernorm(x):
    m = jnp.mean(x, axis=-1, keepdims=True)
    xc = x - m
    v = jnp.mean(xc * xc, axis=-1, keepdims=True)
    return xc * lax.rsqrt(v + EPS)


def _gelu(x):
    c = 0.7978845608028654
    inner = x * (c + (c * 0.044715) * (x * x))
    hx = 0.5 * x
    return hx + hx * jnp.tanh(inner)


def _pack(x):
    return pltpu.bitcast(x.astype(BF16), U32)


def _unpack(x):
    return pltpu.bitcast(x, BF16)


def _recip(x):
    r = pl.reciprocal(x, approx=True)
    return r * (2.0 - x * r)


def _phi(t):
    return jnp.where(t > 0, t + 1.0, jnp.exp(t))


def _kernel(x_hbm, wq_hbm, wk_hbm, wv_hbm, wo_hbm, beta_ref, w1_hbm, w2_hbm, w3_hbm, w4_hbm,
            out_hbm,
            xb, xa, ybuf, hbuf, xoff, wqkv, wo, w1, w2, w3, w4,
            qs, pq, kk, pk, vt, zb, ot, mt, gb, x_sems, qkv_sems, w_sems, out_sems):

    def x_copy(p):
        rows = pl.ds(pl.multiple_of(p * 128, 128), 128)
        return pltpu.make_async_copy(x_hbm.at[0, rows, :], xb.at[rows, :], x_sems.at[p])

    def out_copy(i):
        return pltpu.make_async_copy(xb.at[pl.ds(i * MB, MB), :], out_hbm.at[0, pl.ds(i * MB, MB), :],
                                     out_sems.at[i])

    def qkv_copy(g, i):
        src = (wq_hbm, wk_hbm, wv_hbm)[i]
        return pltpu.make_async_copy(src.at[:, pl.ds(g * 128, 128)],
                                     wqkv.at[g, :, pl.ds(i * 128, 128)], qkv_sems.at[g * 3 + i])

    w_copies = [pltpu.make_async_copy(src, dst, w_sems.at[i])
                for i, (src, dst) in enumerate([(wo_hbm, wo), (w1_hbm, w1), (w2_hbm, w2),
                                                (w3_hbm, w3), (w4_hbm, w4)])]

    x_copy(0).start()
    for i in range(3):
        qkv_copy(0, i).start()
    for p in range(1, NT):
        x_copy(p).start()

    beta = beta_ref[...].astype(F32)
    g_row = 1.0 / (1.0 + jnp.exp(-beta))
    eye = lax.broadcasted_iota(jnp.int32, (H, H), 0) == lax.broadcasted_iota(jnp.int32, (H, H), 1)
    g_col = jnp.sum(jnp.where(eye, g_row, 0.0), axis=1, keepdims=True)
    gb[...] = jnp.broadcast_to(g_col, (H, 128))

    xoff[0] = S
    xoff[1] = S + L
    zero_pad = jnp.zeros((NG, PADR, 128), F32)
    hbuf[:, 0:PADR, :] = zero_pad
    hbuf[:, PADR + S:PADR + S + PADR, :] = zero_pad

    def qkv_tiles(xslot, g, slot):
        xv = xb.at[pl.ds(pl.multiple_of(S + xslot * L, L), L), :]
        wv = wqkv.at[g]
        acc, zacc = {}, []

        def tile(c, n, kt):
            d = _dot(xv[c * 128:(c + 1) * 128, kt * 128:(kt + 1) * 128],
                     wv[kt * 128:(kt + 1) * 128, n * 128:(n + 1) * 128])
            acc[0] = d if kt == 0 else acc[0] + d
            if kt < NG - 1:
                return
            r, rows = acc[0], slice(c * 64, (c + 1) * 64)
            if n == 0:
                qs[slot, rows, :] = _pack(r * QSCALE)
                pq[slot, rows, :] = _pack(_phi(r))
            elif n == 1:
                kk[slot, rows, :] = _pack(r)
                pkf = _phi(r)
                pk[slot, rows, :] = _pack(pkf)
                zacc.append(jnp.sum(pkf.reshape(16, 8, 128), axis=0))
                if c == NT - 1:
                    zb[slot] = jnp.sum(sum(zacc), axis=0, keepdims=True)
            else:
                vt[slot, :, c * 128:(c + 1) * 128] = _pack(r.T)

        return [(128, partial(tile, c, n, kt))
                for c in range(NT) for n in ((0, 1, 2) if c < NT - 1 else (2, 1, 0)) for kt in range(NG)]

    class Group:
        def __init__(self, g, slot):
            self.g, self.slot = g, slot
            self.mem, self.rden, self.parts, self.upd = {}, {}, {}, None
            self.corners, self.outs = {}, {}

        def retrieve(self, j):
            mem = _dot_nt(mt[self.g].astype(BF16), _unpack(pq[self.slot, j * 64:(j + 1) * 64, :]))
            self.mem[j] = mem
            self.rden[j] = _recip(mem[128:136] + 1e-6)

        def update(self, t):
            g, slot = self.g, self.slot
            d = _dot(_unpack(vt[slot, :, t * 128:(t + 1) * 128]), _unpack(pk[slot, t * 64:(t + 1) * 64, :]))
            self.upd = d if t == 0 else self.upd + d
            if t < NT - 1:
                return
            row = lax.broadcasted_iota(jnp.int32, (128, 128), 0)
            col = lax.broadcasted_iota(jnp.int32, (128, 128), 1)
            mt[g, 0:128, :] = mt[g, 0:128, :] + jnp.where(row // DH == col // DH, self.upd, 0.0)
            zrow = lax.broadcasted_iota(jnp.int32, (MROWS - 128, 128), 0)
            zlane = lax.broadcasted_iota(jnp.int32, (MROWS - 128, 128), 1)
            mt[g, 128:MROWS, :] = mt[g, 128:MROWS, :] + jnp.where(zrow == zlane // DH, zb[slot], 0.0)

        def masked_q(self, lo, n, h):
            lane = lax.broadcasted_iota(jnp.int32, (n, 128), 1)
            return jnp.where((lane >= h * DH) & (lane < (h + 1) * DH),
                             qs[self.slot, lo:lo + n, :], jnp.uint32(0))

        def scores(self, j, h):
            self.parts[j, h] = []
            return _dot_nt(_unpack(kk[self.slot, 0:j * 64 + 32, :]), _unpack(self.masked_q(j * 64, 64, h)))

        def corner(self, j, h):
            qc = jnp.concatenate([self.masked_q(j * 64 + 32, 32, h + d) for d in range(2)], axis=0)
            st = _dot_nt(_unpack(kk[self.slot, j * 64 + 32:(j + 1) * 64, :]), _unpack(qc))
            self.corners[j, h] = pltpu.roll(st, 64, 1)
            self.corners[j, h + 1] = st

        def weigh(self, j, h, t, st):
            if t == j:
                st = jnp.concatenate([st[t * 128:t * 128 + 64], self.corners[j, h]], axis=0)
                key_i = lax.broadcasted_iota(jnp.int32, (128, 128), 0)
                qry_i = lax.broadcasted_iota(jnp.int32, (128, 128), 1)
                st = jnp.where(key_i <= qry_i, st, NEG)
            else:
                st = st[t * 128:(t + 1) * 128]
            m = jnp.max(st, axis=0, keepdims=True)
            p = jnp.exp2(st - m)
            l = jnp.sum(p.reshape(16, 8, 128), axis=0)
            pv = _dot(_unpack(vt[self.slot, h * 16:(h + 1) * 16, t * 128:(t + 1) * 128]), p.astype(BF16))
            parts = self.parts[j, h]
            parts.append((m, l, pv))
            if len(parts) < j + 1:
                return
            gate = gb[pl.ds(self.g * HPG + h, 1), :]
            o = self.mem[j][h * DH:(h + 1) * DH] * (gate * self.rden[j][h:h + 1])
            if j == 0:
                o = o + pv * ((1.0 - gate) * _recip(jnp.sum(l, axis=0, keepdims=True)))
            else:
                mx = reduce(jnp.maximum, [pt[0] for pt in parts])
                alphas = [jnp.exp2(pt[0] - mx) for pt in parts]
                lp = sum(al * pt[1] for al, pt in zip(alphas, parts))
                r2 = (1.0 - gate) * _recip(jnp.sum(lp, axis=0, keepdims=True))
                for al, pt in zip(alphas, parts):
                    o = o + pt[2] * (al * r2)
            outs = self.outs.setdefault(j, {})
            outs[h] = o
            if len(outs) == HPG:
                o4 = jnp.concatenate([outs[i] for i in range(HPG)], axis=0)
                ot[self.g, j * 64:(j + 1) * 64, :] = _pack(o4.T)

    def attn_block(groups, fillers):
        free = [0] * 4
        lead, start = [], 0
        for grp in groups:
            for j in range(NT):
                lead.append((start, MROWS, partial(grp.retrieve, j), None))
                for h in range(HPG):
                    dur = 128 * j + 64
                    lead.append((start, dur, partial(grp.scores, j, h), (grp, j, h)))
                    if h % 2 == 0:
                        lead.append((start + max(0, dur - CLEAD), 64, partial(grp.corner, j, h), None))
                    start += int((dur + 32) * RATE)
                    if j == NT - 1:
                        lead.append((start - 256 if grp is not groups[-1] else 10 ** 6, 128,
                                     partial(grp.update, h), None))
        lead.sort(key=lambda e: e[0])
        ready = []
        fillers = list(fillers)

        def issue(dur):
            i = min(range(4), key=lambda m: free[m])
            t0 = free[i]
            free[i] = t0 + dur
            return t0

        while lead or ready or fillers:
            now = min(free)
            if ready and (ready[0][0] <= now or not (lead or fillers)):
                issue(PVD)
                ready.pop(0)[1]()
            elif lead and (lead[0][0] <= now or not fillers):
                _, dur, fn, qk = lead.pop(0)
                t0 = issue(dur)
                res = fn()
                if qk is not None:
                    grp, j, h = qk
                    for t in range(j + 1):
                        ready.append((t0 + min(128 * (t + 1), dur) + DELAY,
                                      partial(grp.weigh, j, h, t, res)))
                    ready.sort(key=lambda e: e[0])
            else:
                dur, fn = fillers.pop(0)
                issue(dur)
                fn()

    def norm_input(src, dst, n):
        xb[pl.ds(dst, n), :] = _layernorm(xb[pl.ds(src, n), :].astype(F32)).astype(BF16)

    for p in range(NT):
        x_copy(p).wait()
    for i in range(3):
        qkv_copy(0, i).wait()
    for g in (1, 2):
        for i in range(3):
            qkv_copy(g, i).start()
    for p in range(NT):
        norm_input(p * 128, S + p * 128, 128)
    for _, c in qkv_tiles(0, 0, 0):
        c()

    def phase_a(t):
        s = t % NSEG
        r0 = pl.multiple_of(s * L, L)
        xslot = t % 2

        @pl.when(s == 0)
        def _():
            mt[...] = jnp.zeros(mt.shape, F32)

        def body(i, c):
            g = 2 * i

            @pl.when(t == 0)
            def _():
                for j in range(3):
                    qkv_copy(g + 1, j).wait()

                @pl.when(i < NG // 2 - 1)
                def _():
                    for j in range(3):
                        qkv_copy(g + 2, j).wait()

                @pl.when(i == 0)
                def _():
                    for g2 in range(3, NG):
                        for j in range(3):
                            qkv_copy(g2, j).start()
                    for p in range(NT, 2 * NT):
                        x_copy(p).start()

                @pl.when(i == 1)
                def _():
                    w_copies[0].start()
                    w_copies[1].start()
                    for p in range(2 * NT, NSEG * NT):
                        x_copy(p).start()

                @pl.when(i == NG // 2 - 1)
                def _():
                    for p in range(NT, 2 * NT):
                        x_copy(p).wait()
                    norm_input(L, S + L, L)

            last = i == NG // 2 - 1
            fa = qkv_tiles(xslot, g + 1, 1)
            fb = qkv_tiles(jnp.where(last, 1 - xslot, xslot), jnp.where(last, 0, g + 2), 0)
            fillers = fa + fb
            attn_block([Group(g, 0), Group(g + 1, 1)], fillers)
            return c
        lax.fori_loop(0, NG // 2, body, 0)

        @pl.when(t == 0)
        def _():
            w_copies[0].wait()
            w_copies[1].wait()
            for p in range(2 * NT, NSEG * NT):
                x_copy(p).wait()
            for c in w_copies[2:]:
                c.start()

        sub = L // SUBA
        hview = hbuf.at[:, pl.ds(r0, L + 2 * PADR), :]
        xv, xav, yv = (r.at[pl.ds(r0, L), :] for r in (xb, xa, ybuf))
        ys = {}

        def op(i):
            rows = slice(i * sub, (i + 1) * sub)
            o = jnp.concatenate([ot[g, i * sub // 2:(i + 1) * sub // 2, :] for g in range(NG)], axis=1)
            x2 = xv[rows, :].astype(F32) + _dot(_unpack(o), wo[...])
            y = _layernorm(x2)
            xav[rows, :] = x2
            yv[rows, :] = y
            ys[i] = _layernorm(y).astype(BF16)

        def up(i):
            hv = _gelu(_dot(ys[i], w1[...]))
            for g in range(NG):
                hview[g, PADR + i * sub:PADR + (i + 1) * sub, :] = hv[:, g * 128:(g + 1) * 128]

        def nrm(i):
            norm_input(pl.multiple_of(((t + 2) % NSEG) * L, L) + i * sub,
                       pl.multiple_of(xoff[xslot], 16) + i * sub, sub)

        for tok in AORD.split(','):
            {'o': op, 'u': up, 'n': nrm}[tok[0]](int(tok[1]))

    def phase_b(t, i):
        tile = (t % NSEG) * (L // MB) + i
        r0 = pl.multiple_of(tile * MB, MB)
        hview = hbuf.at[:, pl.ds(r0, MB + 2 * PADR), :]
        shifts = (-1, -1, 1, 1, -2, -2, 2, 2)
        sub = MB // SUBB
        ts, xn2 = [], []
        for j in range(SUBB):
            rows = pl.ds(r0 + j * sub, sub)
            lo = PADR + j * sub
            hs_in = jnp.concatenate(
                [hview[g, lo + shifts[g]:lo + shifts[g] + sub, :].astype(BF16) for g in range(NG)], axis=1)
            x1 = ybuf[rows, :] + _dot(hs_in, w2[...])
            ts.append(xa[rows, :] + x1)
            xn2.append(_layernorm(x1).astype(BF16))
        ha = jnp.concatenate([_gelu(_dot(v, w3[:, 0:W3A])).astype(BF16) for v in xn2], axis=0)
        hb = _gelu(_dot(jnp.concatenate(xn2, axis=0), w3[:, W3A:F])).astype(BF16)
        h2 = jnp.concatenate([ha, hb], axis=1)
        res = jnp.concatenate(ts, axis=0) + _dot(h2, w4[...])
        xb[pl.ds(r0, MB), :] = res.astype(BF16)

        @pl.when(t >= NSTEP - NSEG)
        def _():
            out_copy(tile).start()

    def step(t, c):
        @pl.when(t < NSTEP)
        def _():
            phase_a(t)

        @pl.when(t == 1)
        def _():
            for cp in w_copies[2:]:
                cp.wait()

        @pl.when(t > 0)
        def _():
            lax.fori_loop(0, L // MB, lambda i, c: (phase_b(t - 1, i), c)[1], 0)
        return c
    lax.fori_loop(0, NSTEP + 1, step, 0)

    for i in range(S // MB):
        out_copy(i).wait()


@jax.jit
def pallas_interleave_layers__memory_aug_infini_attn__mixer_s_mlp__prompt_kernel(
    A_x: jax.Array,
    A_wq: jax.Array,
    A_wk: jax.Array,
    A_wv: jax.Array,
    A_wo: jax.Array,
    A_beta: jax.Array,
    B_x: jax.Array,
    B_w1: jax.Array,
    B_w2: jax.Array,
    B_w3: jax.Array,
    B_w4: jax.Array,
):
    del B_x
    hbm = pl.BlockSpec(memory_space=pl.ANY)
    vmem = pl.BlockSpec(memory_space=pltpu.VMEM)
    scratch = [
        pltpu.VMEM((S + 2 * L, D), BF16),
        pltpu.VMEM((S, D), F32),
        pltpu.VMEM((S, D), F32),
        pltpu.VMEM((NG, S + 2 * PADR, 128), F32),
        pltpu.SMEM((2,), jnp.int32),
        pltpu.VMEM((NG, D, 384), BF16),
        pltpu.VMEM((D, D), BF16),
        pltpu.VMEM((D, D), BF16),
        pltpu.VMEM((D, D), BF16),
        pltpu.VMEM((D, F), BF16),
        pltpu.VMEM((F, D), BF16),
        pltpu.VMEM((2, L // 2, 128), U32),
        pltpu.VMEM((2, L // 2, 128), U32),
        pltpu.VMEM((2, L // 2, 128), U32),
        pltpu.VMEM((2, L // 2, 128), U32),
        pltpu.VMEM((2, 64, L), U32),
        pltpu.VMEM((2, 1, 128), F32),
        pltpu.VMEM((NG, L // 2, 128), U32),
        pltpu.VMEM((NG, MROWS, 128), F32),
        pltpu.VMEM((H, 128), F32),
        pltpu.SemaphoreType.DMA((S // 128,)),
        pltpu.SemaphoreType.DMA((3 * NG,)),
        pltpu.SemaphoreType.DMA((5,)),
        pltpu.SemaphoreType.DMA((S // MB,)),
    ]
    return pl.pallas_call(
        _kernel,
        out_shape=jax.ShapeDtypeStruct(A_x.shape, A_x.dtype),
        in_specs=[hbm, hbm, hbm, hbm, hbm, vmem, hbm, hbm, hbm, hbm],
        out_specs=hbm,
        scratch_shapes=scratch,
        compiler_params=pltpu.CompilerParams(vmem_limit_bytes=120 * 1024 * 1024),
    )(A_x, A_wq, A_wk, A_wv, A_wo, A_beta.reshape(1, H), B_w1, B_w2, B_w3, B_w4)
```

```python
from functools import partial, reduce

import jax
import jax.numpy as jnp
from jax import lax
import jax.experimental.pallas as pl
import jax.experimental.pallas.tpu as pltpu

S = 2048
D = 1024
H = 32
DH = 32
NSEG = 4
NLAYER = 2
NSTEP = NSEG * NLAYER
L = S // NSEG
F = 3584
NG = D // 128
HPG = 128 // DH
NT = L // 128
EPS = 1e-5
LOG2E = 1.4426950408889634
QSCALE = (DH ** -0.5) * LOG2E
NEG = -1e30
PADR = 8
MROWS = 144
MB = 256

SUBA = 4
SUBB = 2
W3A = 768
AORD = 'o0,n0o0,n1o0,o1,l0o1,o2,l1o2,o3,l2o3,u0,l3u0,u1,n2u1,u2,n3u2,u3'
LNC = 16
LUSE = 62
NUSE = 60
BU0 = 52
BU1 = 32
ANC = 1
PRE = 4
PSTEP = '1122300'
RATE = 0.975
NF = 4
UROWS = [32 * int(c) for c in '2222']
DD = 96
SB = 128
CGAP = 8
CMIN = -32
DELAY = 405
PVD = 32
CLEAD = 192
F32 = jnp.float32
BF16 = jnp.bfloat16
U32 = jnp.uint32


def _dot(a, b):
    return jnp.dot(a, b, preferred_element_type=F32)


def _dot_nt(a, b):
    return lax.dot_general(a, b, (((1,), (1,)), ((), ())), preferred_element_type=F32)


def _each(n, fn):
    lax.fori_loop(0, n, lambda i, c: (fn(i), c)[1], 0)


def _rows(ref, lead, start, size):
    if ref.dtype == BF16:
        ref = ref.bitcast(U32)
    return pltpu.bitcast(ref[(*lead, slice(start // 2, (start + size) // 2), slice(None))], BF16)


def _seg(ref, which):
    return ref.bitcast(U32).at[:, pl.ds(pl.multiple_of(which * (L // 2), L // 2), L // 2), :]


def _cols(ref, start, size):
    return jnp.concatenate([_rows(ref, (n,), start, size) for n in range(ref.shape[0])], axis=1)


def _tiled_dot(lhs, w):
    cols, marks = [], []
    for n in range(w.shape[0]):
        for k in range(lhs.shape[1] // 128):
            d = _dot(lhs[:, k * 128:(k + 1) * 128], _rows(w, (n,), k * 128, 128))
            marks.append(d)
            acc = d if k == 0 else acc + d
        cols.append(acc)
    return jnp.concatenate(cols, axis=1), marks


def _put_cols(ref, rows, x):
    for n in range(ref.shape[0]):
        ref[n, rows, :] = x[:, n * 128:(n + 1) * 128]


def _layernorm(x, after=None):
    m = jnp.mean(x, axis=-1, keepdims=True)
    if after is not None:
        m = jnp.concatenate([m + after] * (x.shape[1] // 128), axis=1)
    xc = x - m
    v = jnp.mean(xc * xc, axis=-1, keepdims=True)
    return xc * lax.rsqrt(v + EPS)


def _gelu(x):
    c = 0.7978845608028654
    inner = x * (c + (c * 0.044715) * (x * x))
    hx = 0.5 * x
    return hx + hx * jnp.tanh(inner)


def _unpack(x):
    return pltpu.bitcast(x, BF16)


def _recip(x):
    r = pl.reciprocal(x, approx=True)
    return r * (2.0 - x * r)


def _phi(t):
    return jnp.where(t > 0, t + 1.0, jnp.exp(t))


def _kernel(x_hbm, wq_hbm, wk_hbm, wv_hbm, wo_hbm, beta_hbm, w1_hbm, w2_hbm, w3_hbm, w4_hbm,
            out_hbm,
            xb, xn, xa, ybuf, hbuf, zero, wqkv, wo, w1, w2, w3a, w3, w4,
            qs, pq, kk, pk, vt, zb, ot, mt, gb, beta_ref, x_sems, qkv_sems, w_sems, out_sems):

    def lanes(n):
        return pl.ds(pl.multiple_of(n * 128, 128), 128)

    def x_copy(seg):
        rows = pl.ds(seg * L, L)
        return pltpu.make_async_copy(x_hbm.at[0, rows, :], xb.at[rows, :], x_sems.at[seg + NT - 1])

    def head_copy(p):
        rows = pl.ds(p * 128, 128)
        return pltpu.make_async_copy(x_hbm.at[0, rows, :], xb.at[rows, :], x_sems.at[p])

    beta_copy = pltpu.make_async_copy(beta_hbm, beta_ref, w_sems.at[6])

    def out_copy(i):
        rows = pl.ds(pl.multiple_of(i * MB, MB), MB)
        return pltpu.make_async_copy(xb.at[rows, :], out_hbm.at[0, rows, :], out_sems.at[i])

    def qkv_copy(g, i):
        src = (wq_hbm, wk_hbm, wv_hbm)[i]
        return pltpu.make_async_copy(src.at[:, lanes(g)], wqkv.at[g, i], qkv_sems.at[g * 3 + i])

    def w_copy(i, n):
        src, dst = ((wo_hbm, wo), (w1_hbm, w1), (w2_hbm, w2), (w3_hbm, w3a))[i]
        return pltpu.make_async_copy(src.at[:, lanes(n)], dst.at[n], w_sems.at[i])

    wide_copies = [pltpu.make_async_copy(w3_hbm.at[:, pl.ds(W3A, F - W3A)], w3, w_sems.at[4]),
                   pltpu.make_async_copy(w4_hbm, w4, w_sems.at[5])]

    def start_all(copy, i, n=NG):
        for c in range(n):
            copy(i, c).start()

    def wait_all(copy, i, n=NG):
        for c in range(n):
            copy(i, c).wait()

    early = [head_copy(p) for p in range(NT)] + [qkv_copy(g, i) for g in range(3) for i in range(3)]
    for cp in early[:PRE]:
        cp.start()
    beta_copy.start()

    mt[...] = jnp.zeros(mt.shape, F32)
    zero[0] = 0
    zero_pad = jnp.zeros((NG, PADR, 128), F32)
    hbuf[:, 0:PADR, :] = zero_pad
    hbuf[:, PADR + S:PADR + S + PADR, :] = zero_pad

    def qkv_tiles(xslot, g, slot):
        xv = _seg(xn, xslot)
        acc, zacc = {}, []

        def tile(c, n, kt):
            d = _dot(_rows(xv, (kt,), c * 128, 128), _rows(wqkv, (g, n), kt * 128, 128))
            acc[0] = d if kt == 0 else acc[0] + d
            if kt < NG - 1:
                return
            r, rows = acc[0], slice(c * 128, (c + 1) * 128)
            if n == 0:
                qs[slot, rows, :] = (r * QSCALE).astype(BF16)
                pq[slot, rows, :] = _phi(r).astype(BF16)
            elif n == 1:
                kk[slot, rows, :] = r.astype(BF16)
                pkf = _phi(r)
                pk[slot, rows, :] = pkf.astype(BF16)
                zacc.append(jnp.sum(pkf.reshape(16, 8, 128), axis=0))
                if c == NT - 1:
                    zb[slot] = jnp.sum(sum(zacc), axis=0, keepdims=True)
            else:
                vt[slot, c] = r.T.astype(BF16)

        return [(128, partial(tile, c, n, kt))
                for c in range(NT) for n in ((0, 1, 2) if c < NT - 1 else (2, 1, 0)) for kt in range(NG)]

    class Group:
        def __init__(self, g, slot):
            self.g, self.slot = g, slot
            self.mem, self.rden, self.parts, self.upd = {}, {}, {}, {}
            self.diag, self.outs = {}, {}

        def retrieve(self, j):
            mem = _dot_nt(mt[self.g].astype(BF16), _rows(pq, (self.slot,), j * 128, 128))
            self.mem[j] = mem
            self.rden[j] = _recip(mem[128:136] + 1e-6)

        def update(self, t, lo, n):
            g, slot = self.g, self.slot
            d = _dot(_rows(vt, (slot, t), lo, n), _rows(pk, (slot,), t * 128, 128))
            for r in range(lo, lo + n, DH):
                part = d[r - lo:r - lo + DH]
                self.upd[r] = part if t == 0 else self.upd[r] + part
            if t < NT - 1 or lo + n < 128:
                return
            upd = jnp.concatenate([self.upd[r] for r in range(0, 128, DH)], axis=0)
            row = lax.broadcasted_iota(jnp.int32, (128, 128), 0)
            col = lax.broadcasted_iota(jnp.int32, (128, 128), 1)
            mt[g, 0:128, :] = mt[g, 0:128, :] + jnp.where(row // DH == col // DH, upd, 0.0)
            zrow = lax.broadcasted_iota(jnp.int32, (MROWS - 128, 128), 0)
            zlane = lax.broadcasted_iota(jnp.int32, (MROWS - 128, 128), 1)
            mt[g, 128:MROWS, :] = mt[g, 128:MROWS, :] + jnp.where(zrow == zlane // DH, zb[slot], 0.0)

        def masked_q(self, lo, n, h):
            lane = lax.broadcasted_iota(jnp.int32, (n, 128), 1)
            q = qs.bitcast(U32)[self.slot, lo:lo + n, :]
            return jnp.where((lane >= h * DH) & (lane < (h + 1) * DH), q, jnp.uint32(0))

        def scores(self, j, h):
            self.parts[j, h] = []
            return _dot_nt(_rows(kk, (self.slot,), 0, j * 128 + 32), _unpack(self.masked_q(j * 64, 64, h)))

        def outer(self, j, ha, hb):
            lane = lax.broadcasted_iota(jnp.int32, (16, 128), 1)
            kp = kk.bitcast(U32)
            keys = jnp.where((lane // DH) % 2 == hb % 2, kp[self.slot, j * 64 + 48:j * 64 + 64, :],
                             kp[self.slot, j * 64 + 16:j * 64 + 32, :])
            qc = jnp.concatenate([self.masked_q(j * 64 + 48, 16, hb), self.masked_q(j * 64 + 16, 48, ha)], axis=0)
            st = _dot_nt(_unpack(keys), _unpack(qc))
            self.diag[j, ha, 0] = st
            self.diag[j, hb, 2] = pltpu.roll(st, 96, 1)

        def inner(self, j, h):
            qc = jnp.concatenate([self.masked_q(j * 64 + 32, 32, h + d) for d in range(2)], axis=0)
            st = _dot_nt(_rows(kk, (self.slot,), j * 128 + 64, 32), _unpack(qc))
            self.diag[j, h, 1] = pltpu.roll(st, 64, 1)
            self.diag[j, h + 1, 1] = st

        def weigh(self, j, h, t, st):
            if t == j:
                st = jnp.concatenate([st[t * 128:t * 128 + 32]] + [self.diag[j, h, i] for i in range(3)], axis=0)
                key_i = lax.broadcasted_iota(jnp.int32, (128, 128), 0)
                qry_i = lax.broadcasted_iota(jnp.int32, (128, 128), 1)
                st = jnp.where(key_i <= qry_i, st, NEG)
            else:
                st = st[t * 128:(t + 1) * 128]
            m = jnp.max(st, axis=0, keepdims=True)
            p = jnp.exp2(st - m)
            l = jnp.sum(p.reshape(16, 8, 128), axis=0)
            pv = _dot(_rows(vt, (self.slot, t), h * DH, DH), p.astype(BF16))
            parts = self.parts[j, h]
            parts.append((m, l, pv))
            if len(parts) < j + 1:
                return
            gate = gb[pl.ds(self.g * HPG + h, 1), :]
            o = self.mem[j][h * DH:(h + 1) * DH] * (gate * self.rden[j][h:h + 1])
            if j == 0:
                o = o + pv * ((1.0 - gate) * _recip(jnp.sum(l, axis=0, keepdims=True)))
            else:
                mx = reduce(jnp.maximum, [pt[0] for pt in parts])
                alphas = [jnp.exp2(pt[0] - mx) for pt in parts]
                lp = sum(al * pt[1] for al, pt in zip(alphas, parts))
                r2 = (1.0 - gate) * _recip(jnp.sum(lp, axis=0, keepdims=True))
                for al, pt in zip(alphas, parts):
                    o = o + pt[2] * (al * r2)
            outs = self.outs.setdefault(j, {})
            outs[h] = o
            if len(outs) == HPG:
                o4 = jnp.concatenate([outs[i] for i in range(HPG)], axis=0)
                ot[self.g, j * 128:(j + 1) * 128, :] = o4.T.astype(BF16)

    def attn_block(groups, fillers):
        free = [0] * 4
        lead, start = [], 0
        for grp in groups:
            for j in range(NT):
                lead.append((start, MROWS, partial(grp.retrieve, j), None))
                for h in range(HPG):
                    dur = 128 * j + 32
                    lead.append((start, dur, partial(grp.scores, j, h), (grp, j, h, dur)))
                    if h % 2 == 0:
                        for q, fn in enumerate((partial(grp.outer, j, h + 1, h), partial(grp.inner, j, h),
                                                partial(grp.outer, j, h, h + 1))):
                            lead.append((start + max(CMIN, dur - CLEAD) + q * CGAP, PVD, fn, (grp, j, h, None)))
                    start += int((128 * j + SB) * RATE * 4400 / (3072 + 16 * SB))
                    if j == NT - 1:
                        n = 128 if grp is not groups[-1] else UROWS[h]
                        for lo in range(0, 128, n):
                            lead.append((start - 256 if grp is not groups[-1] else 10 ** 6, n,
                                         partial(grp.update, h, lo, n), None))
        lead.sort(key=lambda e: e[0])
        ready, diag = [], {}
        fillers = list(fillers)

        def issue(dur):
            i = min(range(4), key=lambda m: free[m])
            t0 = free[i]
            free[i] = t0 + dur
            return t0

        for _ in range(NF):
            dur, fn = fillers.pop(0)
            issue(dur)
            fn()
        while lead or ready or fillers:
            now = min(free)
            if ready and (ready[0][0] <= now or not (lead or fillers)):
                issue(PVD)
                ready.pop(0)[1]()
            elif lead and (lead[0][0] <= now or not fillers):
                _, dur, fn, qk = lead.pop(0)
                t0 = issue(dur)
                res = fn()
                if qk is not None:
                    grp, j, h, full = qk
                    if full:
                        ready += [(t0 + 128 * (t + 1) + DELAY, partial(grp.weigh, j, h, t, res)) for t in range(j)]
                    for hd in (h,) if full else (h, h + 1):
                        need = diag.setdefault((grp.slot, j, hd), [])
                        need.append((t0 + dur + (0 if full else DD), res))
                        if len(need) == 4:
                            ready.append((max(e[0] for e in need) + DELAY,
                                          partial(grp.weigh, j, hd, j, [e[1] for e in need if e[1] is not None][0])))
                    ready.sort(key=lambda e: e[0])
            else:
                dur, fn = fillers.pop(0)
                issue(dur)
                fn()

    def norm_input(src, dst, lo, n, after=None):
        x = src[lo:lo + n, :].astype(F32)
        _put_cols(dst, slice(lo, lo + n), _layernorm(x, after).astype(BF16))

    def blank(v):
        return jnp.where(zero[0] != 0, v, 0.0)

    started = [PRE]

    def arrive(k):
        early[k].wait()
        for cp in early[started[0]:started[0] + int(PSTEP[k])]:
            cp.start()
        started[0] += int(PSTEP[k])

    for p in range(NT):
        arrive(p)
        norm_input(xb, xn, p * 128, 128)
    beta_copy.wait()
    beta = beta_ref[...].astype(F32)
    g_row = 1.0 / (1.0 + jnp.exp(-beta))
    eye = lax.broadcasted_iota(jnp.int32, (H, H), 0) == lax.broadcasted_iota(jnp.int32, (H, H), 1)
    g_col = jnp.sum(jnp.where(eye, g_row, 0.0), axis=1, keepdims=True)
    gb[...] = jnp.broadcast_to(g_col, (H, 128))

    first = qkv_tiles(0, 0, 0)
    for i in range(3):
        arrive(NT + i)
        for _, c in first:
            if c.args[1] == i:
                c()

    def phase_a(t):
        s = t % NSEG
        r0 = pl.multiple_of(s * L, L)
        xslot = t % 2

        @pl.when(t == NSEG)
        def _():
            mt[...] = jnp.zeros(mt.shape, F32)

        def body(i, c):
            g = 2 * i

            @pl.when(t == 0)
            def _():
                for j in range(3):
                    qkv_copy(g + 1, j).wait()

                @pl.when(i < NG // 2 - 1)
                def _():
                    for j in range(3):
                        qkv_copy(g + 2, j).wait()

                @pl.when(i == 0)
                def _():
                    for g2 in range(3, NG):
                        for j in range(3):
                            qkv_copy(g2, j).start()
                    x_copy(1).start()

                @pl.when(i == 1)
                def _():
                    start_all(w_copy, 0)
                    start_all(w_copy, 1)
                    x_copy(2).start()
                    x_copy(3).start()

                @pl.when(i == NG // 2 - 1)
                def _():
                    x_copy(1).wait()
                    norm_input(xb, xn, L, L)

            last = i == NG // 2 - 1
            fa = qkv_tiles(xslot, g + 1, 1)
            fb = qkv_tiles(jnp.where(last, 1 - xslot, xslot), jnp.where(last, 0, g + 2), 0)
            attn_block([Group(g, 0), Group(g + 1, 1)], fa + fb)
            return c
        lax.fori_loop(0, NG // 2, body, 0)

        @pl.when(t == 0)
        def _():
            wait_all(w_copy, 0)
            wait_all(w_copy, 1)
            x_copy(2).wait()
            x_copy(3).wait()
            start_all(w_copy, 2)
            start_all(w_copy, 3, W3A // 128)
            for cp in wide_copies:
                cp.start()

        sub = L // SUBA
        hview = hbuf.at[:, pl.ds(r0, L + 2 * PADR), :]
        xav, yv = (r.at[pl.ds(r0, L), :] for r in (xa, ybuf))
        xv, xnext = (xb.at[pl.ds(pl.multiple_of(q * L, L), L), :] for q in (s, (t + 2) % NSEG))
        xnv = xn.at[:, pl.ds(pl.multiple_of(xslot * L, L), L), :]
        ys, x2s, res, pend = {}, {}, {}, []

        def tile_of(dep, k):
            return blank(res[dep][k][0:LNC]) if k >= 0 else None

        def op(i, dep):
            attn, res['o%d' % i] = _tiled_dot(_cols(ot, i * sub, sub), wo)
            x2s[i] = xv[i * sub:(i + 1) * sub, :].astype(F32) + attn
            xav[i * sub:(i + 1) * sub, :] = x2s[i]

        def ln(i, dep):
            zs = []
            for c in range(sub // LNC):
                after = tile_of(dep, (c * LNC * LUSE) // sub - 1)
                if pend and c == ANC:
                    pend.clear()
                    mark = xn.bitcast(U32)[0, pl.ds(pl.multiple_of(zero[0], 8), LNC), :]
                    mark = blank(pltpu.bitcast(mark, F32))
                    after = mark if after is None else after + mark
                y = _layernorm(x2s[i][c * LNC:(c + 1) * LNC], after)
                yv[i * sub + c * LNC:i * sub + (c + 1) * LNC, :] = y
                zs.append(_layernorm(y).astype(BF16))
            ys[i] = jnp.concatenate(zs, axis=0)

        def up(i, dep):
            pre, res['u%d' % i] = _tiled_dot(ys[i], w1)
            _put_cols(hview, slice(PADR + i * sub, PADR + (i + 1) * sub), _gelu(pre))

        toks = AORD.split(',')

        def nrm(i, dep):
            same = [tk for tk in toks if tk[0] == 'n' and tk[2:] == dep]
            pos = same.index('n%d%s' % (i, dep))
            pend.append(i)
            for c in range(0, sub, LNC):
                norm_input(xnext, xnv, i * sub + c, LNC,
                           tile_of(dep, ((pos * sub + c) * NUSE) // (len(same) * sub) - 1))

        for tok in toks:
            {'o': op, 'u': up, 'n': nrm, 'l': ln}[tok[0]](int(tok[1]), tok[2:])

    def phase_b(t, i):
        tile = (t % NSEG) * (L // MB) + i
        r0 = pl.multiple_of(tile * MB, MB)
        hview = hbuf.at[:, pl.ds(r0, MB + 2 * PADR), :]
        shifts = (-1, -1, 1, 1, -2, -2, 2, 2)
        sub = MB // SUBB
        x1s, ts, xn2, has = [], [], [], []

        def norm(x1, marks, use):
            zs = []
            for c in range(0, sub, LNC):
                k = (c * use) // sub - 1
                zs.append(_layernorm(x1[c:c + LNC], blank(marks[k][0:LNC]) if k >= 0 else None).astype(BF16))
            xn2.append(jnp.concatenate(zs, axis=0))

        for j in range(SUBB):
            rows = pl.ds(r0 + j * sub, sub)
            lo = PADR + j * sub
            hs_in = jnp.concatenate(
                [hview[g, lo + shifts[g]:lo + shifts[g] + sub, :].astype(BF16) for g in range(NG)], axis=1)
            hs, marks = _tiled_dot(hs_in, w2)
            x1s.append(ybuf[rows, :] + hs)
            ts.append(xa[rows, :] + x1s[j])
        norm(x1s[0], marks, BU0)
        pre, marks = _tiled_dot(xn2[0], w3a)
        has.append(_gelu(pre).astype(BF16))
        norm(x1s[1], marks, BU1)
        has.append(_gelu(_tiled_dot(xn2[1], w3a)[0]).astype(BF16))
        ha = jnp.concatenate(has, axis=0)
        hb = _gelu(_dot(jnp.concatenate(xn2, axis=0), w3[...])).astype(BF16)
        h2 = jnp.concatenate([ha, hb], axis=1)
        res = jnp.concatenate(ts, axis=0) + _dot(h2, w4[...])
        xb[pl.ds(r0, MB), :] = res.astype(BF16)

        @pl.when(t >= NSTEP - NSEG)
        def _():
            out_copy(tile).start()

    def step(t, c):
        @pl.when(t < NSTEP)
        def _():
            phase_a(t)

        @pl.when(t == 1)
        def _():
            wait_all(w_copy, 2)
            wait_all(w_copy, 3, W3A // 128)
            for cp in wide_copies:
                cp.wait()

        @pl.when(t > 0)
        def _():
            _each(L // MB, lambda i: phase_b(t - 1, i))
        return c
    lax.fori_loop(0, NSTEP + 1, step, 0)

    for i in range(S // MB):
        out_copy(i).wait()


@jax.jit
def pallas_interleave_layers__memory_aug_infini_attn__mixer_s_mlp__prompt_kernel(
    A_x: jax.Array,
    A_wq: jax.Array,
    A_wk: jax.Array,
    A_wv: jax.Array,
    A_wo: jax.Array,
    A_beta: jax.Array,
    B_x: jax.Array,
    B_w1: jax.Array,
    B_w2: jax.Array,
    B_w3: jax.Array,
    B_w4: jax.Array,
):
    del B_x
    hbm = pl.BlockSpec(memory_space=pl.ANY)
    scratch = [
        pltpu.VMEM((S, D), BF16),
        pltpu.VMEM((NG, 2 * L, 128), BF16),
        pltpu.VMEM((S, D), F32),
        pltpu.VMEM((S, D), F32),
        pltpu.VMEM((NG, S + 2 * PADR, 128), F32),
        pltpu.SMEM((1,), jnp.int32),
        pltpu.VMEM((NG, 3, D, 128), BF16),
        pltpu.VMEM((NG, D, 128), BF16),
        pltpu.VMEM((NG, D, 128), BF16),
        pltpu.VMEM((NG, D, 128), BF16),
        pltpu.VMEM((W3A // 128, D, 128), BF16),
        pltpu.VMEM((D, F - W3A), BF16),
        pltpu.VMEM((F, D), BF16),
        pltpu.VMEM((2, L, 128), BF16),
        pltpu.VMEM((2, L, 128), BF16),
        pltpu.VMEM((2, L, 128), BF16),
        pltpu.VMEM((2, L, 128), BF16),
        pltpu.VMEM((2, NT, 128, 128), BF16),
        pltpu.VMEM((2, 1, 128), F32),
        pltpu.VMEM((NG, L, 128), BF16),
        pltpu.VMEM((NG, MROWS, 128), F32),
        pltpu.VMEM((H, 128), F32),
        pltpu.VMEM((1, H), BF16),
        pltpu.SemaphoreType.DMA((NSEG + NT - 1,)),
        pltpu.SemaphoreType.DMA((3 * NG,)),
        pltpu.SemaphoreType.DMA((7,)),
        pltpu.SemaphoreType.DMA((S // MB,)),
    ]
    return pl.pallas_call(
        _kernel,
        out_shape=jax.ShapeDtypeStruct(A_x.shape, A_x.dtype),
        in_specs=[hbm] * 10,
        out_specs=hbm,
        scratch_shapes=scratch,
        compiler_params=pltpu.CompilerParams(vmem_limit_bytes=120 * 1024 * 1024),
    )(A_x, A_wq, A_wk, A_wv, A_wo, A_beta.reshape(1, H), B_w1, B_w2, B_w3, B_w4)
```

```python
from functools import partial, reduce

import jax
import jax.numpy as jnp
from jax import lax
import jax.experimental.pallas as pl
import jax.experimental.pallas.tpu as pltpu

S = 2048
D = 1024
H = 32
DH = 32
NSEG = 4
NLAYER = 2
NSTEP = NSEG * NLAYER
L = S // NSEG
F = 3584
NG = D // 128
HPG = 128 // DH
NT = L // 128
EPS = 1e-5
LOG2E = 1.4426950408889634
QSCALE = (DH ** -0.5) * LOG2E
NEG = -1e30
PADR = 8
MROWS = 144
MB = 256

SUBA = 4
SUBB = 2
W3A = 768
AORD = 'o0,n0o0,n1o0,o1,l0o1,o2,l1o2,o3,l2o3,u0,l3u0,u1,n2u1,u2,n3u2,u3'
LNC = 16
LUSE = 62
NUSE = 60
BU0 = 52
BU1 = 32
ANC = 1
PORD = 'x0,w0|x1,w1|w2|x2||w3,x3|w4,w5,w6|w7,w8'
XP = 1
XL = 256
RATE = 0.975
RATEF = 0.7
GSL = 12
NF = 4
UROWS = [32 * int(c) for c in '2222']
DD = 96
SB = 128
CGAP = 8
CMIN = -32
DELAY = 405
PVD = 32
CLEAD = 192
F32 = jnp.float32
BF16 = jnp.bfloat16
U32 = jnp.uint32


def _dot(a, b):
    return jnp.dot(a, b, preferred_element_type=F32)


def _dot_nt(a, b):
    return lax.dot_general(a, b, (((1,), (1,)), ((), ())), preferred_element_type=F32)


def _each(n, fn):
    lax.fori_loop(0, n, lambda i, c: (fn(i), c)[1], 0)


def _rows(ref, lead, start, size):
    if ref.dtype == BF16:
        ref = ref.bitcast(U32)
    return pltpu.bitcast(ref[(*lead, slice(start // 2, (start + size) // 2), slice(None))], BF16)


def _seg(ref, which):
    return ref.bitcast(U32).at[:, pl.ds(pl.multiple_of(which * (L // 2), L // 2), L // 2), :]


def _cols(ref, start, size):
    return jnp.concatenate([_rows(ref, (n,), start, size) for n in range(ref.shape[0])], axis=1)


def _tiled_dot(lhs, w):
    cols, marks = [], []
    for n in range(w.shape[0]):
        for k in range(lhs.shape[1] // 128):
            d = _dot(lhs[:, k * 128:(k + 1) * 128], _rows(w, (n,), k * 128, 128))
            marks.append(d)
            acc = d if k == 0 else acc + d
        cols.append(acc)
    return jnp.concatenate(cols, axis=1), marks


def _put_cols(ref, rows, x):
    for n in range(ref.shape[0]):
        ref[n, rows, :] = x[:, n * 128:(n + 1) * 128]


def _layernorm(x, after=None):
    m = jnp.mean(x, axis=-1, keepdims=True)
    if after is not None:
        m = jnp.concatenate([m + after] * (x.shape[1] // 128), axis=1)
    xc = x - m
    v = jnp.mean(xc * xc, axis=-1, keepdims=True)
    return xc * lax.rsqrt(v + EPS)


def _gelu(x):
    c = 0.7978845608028654
    inner = x * (c + (c * 0.044715) * (x * x))
    hx = 0.5 * x
    return hx + hx * jnp.tanh(inner)


def _unpack(x):
    return pltpu.bitcast(x, BF16)


def _recip(x):
    r = pl.reciprocal(x, approx=True)
    return r * (2.0 - x * r)


def _phi(t):
    return jnp.where(t > 0, t + 1.0, jnp.exp(t))


def _kernel(x_hbm, wq_hbm, wk_hbm, wv_hbm, wo_hbm, beta_hbm, w1_hbm, w2_hbm, w3_hbm, w4_hbm,
            out_hbm,
            xb, xn, xa, ybuf, hbuf, zero, wqkv, wo, w1, w2, w3a, w3, w4,
            qs, pq, kk, pk, vt, zb, ot, mt, gb, beta_ref, x_sems, qkv_sems, w_sems, out_sems):

    def lanes(n):
        return pl.ds(pl.multiple_of(n * 128, 128), 128)

    def x_copy(seg):
        rows = pl.ds(seg * L, L)
        return pltpu.make_async_copy(x_hbm.at[0, rows, :], xb.at[rows, :], x_sems.at[seg + NT - 1])

    def head_copy(p):
        return pltpu.make_async_copy(x_hbm.at[0, lanes(p), :], xb.at[lanes(p), :], x_sems.at[p])

    beta_copy = pltpu.make_async_copy(beta_hbm, beta_ref, w_sems.at[6])

    def out_copy(i):
        rows = pl.ds(pl.multiple_of(i * MB, MB), MB)
        return pltpu.make_async_copy(xb.at[rows, :], out_hbm.at[0, rows, :], out_sems.at[i])

    def qkv_copy(g, i):
        src = (wq_hbm, wk_hbm, wv_hbm)[i]
        return pltpu.make_async_copy(src.at[:, lanes(g)], wqkv.at[g, i], qkv_sems.at[g * 3 + i])

    def w_copy(i, n):
        src, dst = ((wo_hbm, wo), (w1_hbm, w1), (w2_hbm, w2), (w3_hbm, w3a))[i]
        return pltpu.make_async_copy(src.at[:, lanes(n)], dst.at[n], w_sems.at[i])

    wide_copies = [pltpu.make_async_copy(w3_hbm.at[:, pl.ds(W3A, F - W3A)], w3, w_sems.at[4]),
                   pltpu.make_async_copy(w4_hbm, w4, w_sems.at[5])]

    def start_all(copy, i, n=NG):
        for c in range(n):
            copy(i, c).start()

    def wait_all(copy, i, n=NG):
        for c in range(n):
            copy(i, c).wait()

    def launch(k):
        for tok in filter(None, PORD.split('|')[k].split(',')):
            n = int(tok[1])
            (head_copy(n) if tok[0] == 'x' else qkv_copy(n // 3, n % 3)).start()

    launch(0)
    beta_copy.start()

    mt[...] = jnp.zeros(mt.shape, F32)
    zero[0] = 0
    zero_pad = jnp.zeros((NG, PADR, 128), F32)
    hbuf[:, 0:PADR, :] = zero_pad
    hbuf[:, PADR + S:PADR + S + PADR, :] = zero_pad

    def project(slot, n, r, rows, c, memory=True):
        if n == 0:
            qs[slot, rows, :] = (r * QSCALE).astype(BF16)
            pq[slot, rows, :] = _phi(r).astype(BF16)
        elif n == 1:
            kk[slot, rows, :] = r.astype(BF16)
            if not memory:
                return []
            pkf = _phi(r)
            pk[slot, rows, :] = pkf.astype(BF16)
            return [jnp.sum(pkf.reshape(16, 8, 128), axis=0)]
        else:
            vt[slot, c] = r.T.astype(BF16)
        return []

    def qkv_tiles(xslot, g, slot, memory=True):
        xv = _seg(xn, xslot)
        acc, zacc = {}, []

        def tile(c, n, kt):
            d = _dot(_rows(xv, (kt,), c * 128, 128), _rows(wqkv, (g, n), kt * 128, 128))
            acc[0] = d if kt == 0 else acc[0] + d
            if kt < NG - 1:
                return
            zacc.extend(project(slot, n, acc[0], slice(c * 128, (c + 1) * 128), c, memory))
            if n == 1 and c == NT - 1 and memory:
                zb[slot] = jnp.sum(sum(zacc), axis=0, keepdims=True)

        return [(128, partial(tile, c, n, kt))
                for c in range(NT) for n in ((0, 1, 2) if c < NT - 1 else (2, 1, 0)) for kt in range(NG)]

    class Group:
        def __init__(self, g, slot):
            self.g, self.slot = g, slot
            self.mem, self.rden, self.parts, self.upd = {}, {}, {}, {}
            self.diag, self.outs = {}, {}

        def retrieve(self, j):
            mem = _dot_nt(mt[self.g].astype(BF16), _rows(pq, (self.slot,), j * 128, 128))
            self.mem[j] = mem
            self.rden[j] = _recip(mem[128:136] + 1e-6)

        def update(self, t, lo, n):
            g, slot = self.g, self.slot
            d = _dot(_rows(vt, (slot, t), lo, n), _rows(pk, (slot,), t * 128, 128))
            for r in range(lo, lo + n, DH):
                part = d[r - lo:r - lo + DH]
                self.upd[r] = part if t == 0 else self.upd[r] + part
            if t < NT - 1 or lo + n < 128:
                return
            upd = jnp.concatenate([self.upd[r] for r in range(0, 128, DH)], axis=0)
            row = lax.broadcasted_iota(jnp.int32, (128, 128), 0)
            col = lax.broadcasted_iota(jnp.int32, (128, 128), 1)
            mt[g, 0:128, :] = mt[g, 0:128, :] + jnp.where(row // DH == col // DH, upd, 0.0)
            zrow = lax.broadcasted_iota(jnp.int32, (MROWS - 128, 128), 0)
            zlane = lax.broadcasted_iota(jnp.int32, (MROWS - 128, 128), 1)
            mt[g, 128:MROWS, :] = mt[g, 128:MROWS, :] + jnp.where(zrow == zlane // DH, zb[slot], 0.0)

        def masked_q(self, lo, n, h):
            lane = lax.broadcasted_iota(jnp.int32, (n, 128), 1)
            q = qs.bitcast(U32)[self.slot, lo:lo + n, :]
            return jnp.where((lane >= h * DH) & (lane < (h + 1) * DH), q, jnp.uint32(0))

        def scores(self, j, h):
            self.parts[j, h] = []
            return _dot_nt(_rows(kk, (self.slot,), 0, j * 128 + 32), _unpack(self.masked_q(j * 64, 64, h)))

        def outer(self, j, ha, hb):
            lane = lax.broadcasted_iota(jnp.int32, (16, 128), 1)
            kp = kk.bitcast(U32)
            keys = jnp.where((lane // DH) % 2 == hb % 2, kp[self.slot, j * 64 + 48:j * 64 + 64, :],
                             kp[self.slot, j * 64 + 16:j * 64 + 32, :])
            qc = jnp.concatenate([self.masked_q(j * 64 + 48, 16, hb), self.masked_q(j * 64 + 16, 48, ha)], axis=0)
            st = _dot_nt(_unpack(keys), _unpack(qc))
            self.diag[j, ha, 0] = st
            self.diag[j, hb, 2] = pltpu.roll(st, 96, 1)

        def inner(self, j, h):
            qc = jnp.concatenate([self.masked_q(j * 64 + 32, 32, h + d) for d in range(2)], axis=0)
            st = _dot_nt(_rows(kk, (self.slot,), j * 128 + 64, 32), _unpack(qc))
            self.diag[j, h, 1] = pltpu.roll(st, 64, 1)
            self.diag[j, h + 1, 1] = st

        def weigh(self, j, h, t, st):
            if t == j:
                st = jnp.concatenate([st[t * 128:t * 128 + 32]] + [self.diag[j, h, i] for i in range(3)], axis=0)
                key_i = lax.broadcasted_iota(jnp.int32, (128, 128), 0)
                qry_i = lax.broadcasted_iota(jnp.int32, (128, 128), 1)
                st = jnp.where(key_i <= qry_i, st, NEG)
            else:
                st = st[t * 128:(t + 1) * 128]
            m = jnp.max(st, axis=0, keepdims=True)
            p = jnp.exp2(st - m)
            l = jnp.sum(p.reshape(16, 8, 128), axis=0)
            pv = _dot(_rows(vt, (self.slot, t), h * DH, DH), p.astype(BF16))
            parts = self.parts[j, h]
            parts.append((m, l, pv))
            if len(parts) < j + 1:
                return
            gate = gb[pl.ds(self.g * HPG + h, 1), :]
            o = self.mem[j][h * DH:(h + 1) * DH] * (gate * self.rden[j][h:h + 1])
            if j == 0:
                o = o + pv * ((1.0 - gate) * _recip(jnp.sum(l, axis=0, keepdims=True)))
            else:
                mx = reduce(jnp.maximum, [pt[0] for pt in parts])
                alphas = [jnp.exp2(pt[0] - mx) for pt in parts]
                lp = sum(al * pt[1] for al, pt in zip(alphas, parts))
                r2 = (1.0 - gate) * _recip(jnp.sum(lp, axis=0, keepdims=True))
                for al, pt in zip(alphas, parts):
                    o = o + pt[2] * (al * r2)
            outs = self.outs.setdefault(j, {})
            outs[h] = o
            if len(outs) == HPG:
                o4 = jnp.concatenate([outs[i] for i in range(HPG)], axis=0)
                ot[self.g, j * 128:(j + 1) * 128, :] = o4.T.astype(BF16)

    def attn_block(groups, fillers, final=False):
        free = [0] * 4
        rate = RATEF if final else RATE
        lead, start = [], 0
        for grp in groups:
            for j in range(NT):
                lead.append((start, MROWS, partial(grp.retrieve, j), None))
                for h in range(HPG):
                    dur = 128 * j + 32
                    lead.append((start, dur, partial(grp.scores, j, h), (grp, j, h, dur)))
                    if h % 2 == 0:
                        for q, fn in enumerate((partial(grp.outer, j, h + 1, h), partial(grp.inner, j, h),
                                                partial(grp.outer, j, h, h + 1))):
                            lead.append((start + max(CMIN, dur - CLEAD) + q * CGAP, PVD, fn, (grp, j, h, None)))
                    start += int((128 * j + SB) * rate * 4400 / (3072 + 16 * SB))
                    if j == NT - 1 and not final:
                        n = 128 if grp is not groups[-1] else UROWS[h]
                        for lo in range(0, 128, n):
                            lead.append((start - 256 if grp is not groups[-1] else 10 ** 6, n,
                                         partial(grp.update, h, lo, n), None))
        lead.sort(key=lambda e: e[0])
        ready, diag = [], {}
        fillers = list(fillers)
        total = len(fillers)

        def fed(fn):
            if not final or fn.func.__self__ is not groups[-1]:
                return True
            return total - len(fillers) >= min(total, 3 * NG * (fn.args[0] + 1) + GSL)

        def issue(dur):
            i = min(range(4), key=lambda m: free[m])
            t0 = free[i]
            free[i] = t0 + dur
            return t0

        for _ in range(NF):
            dur, fn = fillers.pop(0)
            issue(dur)
            fn()
        while lead or ready or fillers:
            now = min(free)
            if ready and (ready[0][0] <= now or not (lead or fillers)):
                issue(PVD)
                ready.pop(0)[1]()
            elif final and not fillers and lead[0][0] > now:
                free[free.index(now)] = min([lead[0][0]] + [e[0] for e in ready[:1]])
            elif lead and (lead[0][0] <= now or not fillers) and fed(lead[0][2]):
                _, dur, fn, qk = lead.pop(0)
                t0 = issue(dur)
                res = fn()
                if qk is not None:
                    grp, j, h, full = qk
                    if full:
                        ready += [(t0 + 128 * (t + 1) + DELAY, partial(grp.weigh, j, h, t, res)) for t in range(j)]
                    for hd in (h,) if full else (h, h + 1):
                        need = diag.setdefault((grp.slot, j, hd), [])
                        need.append((t0 + dur + (0 if full else DD), res))
                        if len(need) == 4:
                            ready.append((max(e[0] for e in need) + DELAY,
                                          partial(grp.weigh, j, hd, j, [e[1] for e in need if e[1] is not None][0])))
                    ready.sort(key=lambda e: e[0])
            else:
                dur, fn = fillers.pop(0)
                issue(dur)
                fn()

    def norm_input(src, dst, lo, n, after=None):
        x = src[lo:lo + n, :].astype(F32)
        _put_cols(dst, slice(lo, lo + n), _layernorm(x, after).astype(BF16))

    def blank(v):
        return jnp.where(zero[0] != 0, v, 0.0)

    def norm_tile(lo, n):
        rows = pl.ds(pl.multiple_of(lo, n), n)
        norm_input(xb.at[rows, :], xn.at[:, rows, :], 0, n)

    head_copy(0).wait()
    launch(1)
    norm_input(xb, xn, 0, 128)
    beta_copy.wait()
    beta = beta_ref[...].astype(F32)
    g_row = 1.0 / (1.0 + jnp.exp(-beta))
    eye = lax.broadcasted_iota(jnp.int32, (H, H), 0) == lax.broadcasted_iota(jnp.int32, (H, H), 1)
    g_col = jnp.sum(jnp.where(eye, g_row, 0.0), axis=1, keepdims=True)
    gb[...] = jnp.broadcast_to(g_col, (H, 128))

    def first(p, z, arrive=None):
        lhs = xn.bitcast(U32).at[:, pl.ds(pl.multiple_of(p * 64, 64), 64), :]
        for n in range(3):
            if arrive:
                arrive(n)
            r, _ = _tiled_dot(_cols(lhs, 0, 128), wqkv.bitcast(U32).at[0, pl.ds(n, 1)])
            z = sum(project(0, n, r, lanes(p), p), z)
        return z

    def weights(n):
        qkv_copy(0, n).wait()
        launch(2 + n)
        if n == XP:
            head_copy(1).wait()
            launch(5)
            norm_input(xb, xn, 128, 128)

    def rest(p, z):
        for q in range(1, NT - 1):
            @pl.when(p == q)
            def _():
                head_copy(q + 1).wait()
                launch(5 + q)
        z = first(p, z)
        norm_tile(jnp.minimum(p + 1, NT - 1) * 128, 128)
        return z
    z0 = first(0, jnp.zeros((8, 128), F32), weights)
    zb[0] = jnp.sum(lax.fori_loop(1, NT, rest, z0), axis=0, keepdims=True)

    def phase_a(t):
        s = t % NSEG
        r0 = pl.multiple_of(s * L, L)
        xslot = t % 2

        @pl.when(t == NSEG)
        def _():
            mt[...] = jnp.zeros(mt.shape, F32)

        def body(i, c):
            g = 2 * i

            @pl.when(t == 0)
            def _():
                for j in range(3):
                    qkv_copy(g + 1, j).wait()

                @pl.when(i < NG // 2 - 1)
                def _():
                    for j in range(3):
                        qkv_copy(g + 2, j).wait()

                @pl.when(i == 0)
                def _():
                    for g2 in range(3, NG):
                        for j in range(3):
                            qkv_copy(g2, j).start()
                    x_copy(1).start()

                @pl.when(i == 1)
                def _():
                    start_all(w_copy, 0)
                    start_all(w_copy, 1)
                    x_copy(2).start()
                    x_copy(3).start()

                @pl.when(i == NG // 2 - 1)
                def _():
                    x_copy(1).wait()
                    _each(L // XL, lambda p: norm_tile(L + p * XL, XL))

            last = i == NG // 2 - 1
            fa = qkv_tiles(xslot, g + 1, 1)
            fb = qkv_tiles(jnp.where(last, 1 - xslot, xslot), jnp.where(last, 0, g + 2), 0)
            attn_block([Group(g, 0), Group(g + 1, 1)], fa + fb)
            return c
        lax.fori_loop(0, jnp.where(t == NSTEP - 1, NG // 2 - 1, NG // 2), body, 0)

        @pl.when(t == NSTEP - 1)
        def _():
            attn_block([Group(NG - 2, 0), Group(NG - 1, 1)], qkv_tiles((NSTEP - 1) % 2, NG - 1, 1, False), True)

        @pl.when(t == 0)
        def _():
            wait_all(w_copy, 0)
            wait_all(w_copy, 1)
            x_copy(2).wait()
            x_copy(3).wait()
            start_all(w_copy, 2)
            start_all(w_copy, 3, W3A // 128)
            for cp in wide_copies:
                cp.start()

        sub = L // SUBA
        hview = hbuf.at[:, pl.ds(r0, L + 2 * PADR), :]
        xav, yv = (r.at[pl.ds(r0, L), :] for r in (xa, ybuf))
        xv, xnext = (xb.at[pl.ds(pl.multiple_of(q * L, L), L), :] for q in (s, (t + 2) % NSEG))
        xnv = xn.at[:, pl.ds(pl.multiple_of(xslot * L, L), L), :]
        ys, x2s, res, pend = {}, {}, {}, []

        def tile_of(dep, k):
            return blank(res[dep][k][0:LNC]) if k >= 0 else None

        def op(i, dep):
            attn, res['o%d' % i] = _tiled_dot(_cols(ot, i * sub, sub), wo)
            x2s[i] = xv[i * sub:(i + 1) * sub, :].astype(F32) + attn
            xav[i * sub:(i + 1) * sub, :] = x2s[i]

        def ln(i, dep):
            zs = []
            for c in range(sub // LNC):
                after = tile_of(dep, (c * LNC * LUSE) // sub - 1)
                if pend and c == ANC:
                    pend.clear()
                    mark = xn.bitcast(U32)[0, pl.ds(pl.multiple_of(zero[0], 8), LNC), :]
                    mark = blank(pltpu.bitcast(mark, F32))
                    after = mark if after is None else after + mark
                y = _layernorm(x2s[i][c * LNC:(c + 1) * LNC], after)
                yv[i * sub + c * LNC:i * sub + (c + 1) * LNC, :] = y
                zs.append(_layernorm(y).astype(BF16))
            ys[i] = jnp.concatenate(zs, axis=0)

        def up(i, dep):
            pre, res['u%d' % i] = _tiled_dot(ys[i], w1)
            _put_cols(hview, slice(PADR + i * sub, PADR + (i + 1) * sub), _gelu(pre))

        toks = AORD.split(',')

        def nrm(i, dep):
            same = [tk for tk in toks if tk[0] == 'n' and tk[2:] == dep]
            pos = same.index('n%d%s' % (i, dep))
            pend.append(i)
            for c in range(0, sub, LNC):
                norm_input(xnext, xnv, i * sub + c, LNC,
                           tile_of(dep, ((pos * sub + c) * NUSE) // (len(same) * sub) - 1))

        for tok in toks:
            {'o': op, 'u': up, 'n': nrm, 'l': ln}[tok[0]](int(tok[1]), tok[2:])

    def phase_b(t, i):
        tile = (t % NSEG) * (L // MB) + i
        r0 = pl.multiple_of(tile * MB, MB)
        hview = hbuf.at[:, pl.ds(r0, MB + 2 * PADR), :]
        shifts = (-1, -1, 1, 1, -2, -2, 2, 2)
        sub = MB // SUBB
        x1s, ts, xn2, has = [], [], [], []

        def norm(x1, marks, use):
            zs = []
            for c in range(0, sub, LNC):
                k = (c * use) // sub - 1
                zs.append(_layernorm(x1[c:c + LNC], blank(marks[k][0:LNC]) if k >= 0 else None).astype(BF16))
            xn2.append(jnp.concatenate(zs, axis=0))

        for j in range(SUBB):
            rows = pl.ds(r0 + j * sub, sub)
            lo = PADR + j * sub
            hs_in = jnp.concatenate(
                [hview[g, lo + shifts[g]:lo + shifts[g] + sub, :].astype(BF16) for g in range(NG)], axis=1)
            hs, marks = _tiled_dot(hs_in, w2)
            x1s.append(ybuf[rows, :] + hs)
            ts.append(xa[rows, :] + x1s[j])
        norm(x1s[0], marks, BU0)
        pre, marks = _tiled_dot(xn2[0], w3a)
        has.append(_gelu(pre).astype(BF16))
        norm(x1s[1], marks, BU1)
        has.append(_gelu(_tiled_dot(xn2[1], w3a)[0]).astype(BF16))
        ha = jnp.concatenate(has, axis=0)
        hb = _gelu(_dot(jnp.concatenate(xn2, axis=0), w3[...])).astype(BF16)
        h2 = jnp.concatenate([ha, hb], axis=1)
        res = jnp.concatenate(ts, axis=0) + _dot(h2, w4[...])
        xb[pl.ds(r0, MB), :] = res.astype(BF16)

        @pl.when(t >= NSTEP - NSEG)
        def _():
            out_copy(tile).start()

    def step(t, c):
        @pl.when(t < NSTEP)
        def _():
            phase_a(t)

        @pl.when(t == 1)
        def _():
            wait_all(w_copy, 2)
            wait_all(w_copy, 3, W3A // 128)
            for cp in wide_copies:
                cp.wait()

        @pl.when(t > 0)
        def _():
            _each(L // MB, lambda i: phase_b(t - 1, i))
        return c
    lax.fori_loop(0, NSTEP + 1, step, 0)

    for i in range(S // MB):
        out_copy(i).wait()


@jax.jit
def pallas_interleave_layers__memory_aug_infini_attn__mixer_s_mlp__prompt_kernel(
    A_x: jax.Array,
    A_wq: jax.Array,
    A_wk: jax.Array,
    A_wv: jax.Array,
    A_wo: jax.Array,
    A_beta: jax.Array,
    B_x: jax.Array,
    B_w1: jax.Array,
    B_w2: jax.Array,
    B_w3: jax.Array,
    B_w4: jax.Array,
):
    del B_x
    hbm = pl.BlockSpec(memory_space=pl.ANY)
    scratch = [
        pltpu.VMEM((S, D), BF16),
        pltpu.VMEM((NG, 2 * L, 128), BF16),
        pltpu.VMEM((S, D), F32),
        pltpu.VMEM((S, D), F32),
        pltpu.VMEM((NG, S + 2 * PADR, 128), F32),
        pltpu.SMEM((1,), jnp.int32),
        pltpu.VMEM((NG, 3, D, 128), BF16),
        pltpu.VMEM((NG, D, 128), BF16),
        pltpu.VMEM((NG, D, 128), BF16),
        pltpu.VMEM((NG, D, 128), BF16),
        pltpu.VMEM((W3A // 128, D, 128), BF16),
        pltpu.VMEM((D, F - W3A), BF16),
        pltpu.VMEM((F, D), BF16),
        pltpu.VMEM((2, L, 128), BF16),
        pltpu.VMEM((2, L, 128), BF16),
        pltpu.VMEM((2, L, 128), BF16),
        pltpu.VMEM((2, L, 128), BF16),
        pltpu.VMEM((2, NT, 128, 128), BF16),
        pltpu.VMEM((2, 1, 128), F32),
        pltpu.VMEM((NG, L, 128), BF16),
        pltpu.VMEM((NG, MROWS, 128), F32),
        pltpu.VMEM((H, 128), F32),
        pltpu.VMEM((1, H), BF16),
        pltpu.SemaphoreType.DMA((NSEG + NT - 1,)),
        pltpu.SemaphoreType.DMA((3 * NG,)),
        pltpu.SemaphoreType.DMA((7,)),
        pltpu.SemaphoreType.DMA((S // MB,)),
    ]
    return pl.pallas_call(
        _kernel,
        out_shape=jax.ShapeDtypeStruct(A_x.shape, A_x.dtype),
        in_specs=[hbm] * 10,
        out_specs=hbm,
        scratch_shapes=scratch,
        compiler_params=pltpu.CompilerParams(vmem_limit_bytes=120 * 1024 * 1024),
    )(A_x, A_wq, A_wk, A_wv, A_wo, A_beta.reshape(1, H), B_w1, B_w2, B_w3, B_w4)
```

```python
from functools import partial, reduce

import jax
import jax.numpy as jnp
from jax import lax
import jax.experimental.pallas as pl
import jax.experimental.pallas.tpu as pltpu

S = 2048
D = 1024
H = 32
DH = 32
NSEG = 4
NLAYER = 2
NSTEP = NSEG * NLAYER
L = S // NSEG
F = 3584
NG = D // 128
HPG = 128 // DH
NT = L // 128
EPS = 1e-5
LOG2E = 1.4426950408889634
QSCALE = (DH ** -0.5) * LOG2E
NEG = -1e30
PADR = 8
MROWS = 144
MB = 256

SUBA = 4
SUBB = 2
W3A = 768
AORD = 'o0,n0o0,n1o0,o1,l0o1,o2,l1o2,u0,l2u0,o3,n2o3,u1,l3u1,u2,n3u2,u3'
LNC = 16
LUSE = 64
NUSE = 66
BU0 = 52
BU1 = 29
ANC = 1
PORD = 'x0,w0|x1,w1|w2|x2||w3,x3|w4,w5,w6|w7,w8'
XP = 1
XL = 256
RATE = 0.975
RATEF = 0.8
GSL = 30
NF = 4
UROWS = [32 * int(c) for c in '2222']
DD = 96
SB = 128
CGAP = 8
CMIN = -32
DELAY = 385
PVD = 32
CLEAD = 192
F32 = jnp.float32
BF16 = jnp.bfloat16
U32 = jnp.uint32


def _dot(a, b):
    return jnp.dot(a, b, preferred_element_type=F32)


def _dot_nt(a, b):
    return lax.dot_general(a, b, (((1,), (1,)), ((), ())), preferred_element_type=F32)


def _each(n, fn):
    lax.fori_loop(0, n, lambda i, c: (fn(i), c)[1], 0)


def _rows(ref, lead, start, size):
    if ref.dtype == BF16:
        ref = ref.bitcast(U32)
    return pltpu.bitcast(ref[(*lead, slice(start // 2, (start + size) // 2), slice(None))], BF16)


def _seg(ref, which):
    return ref.bitcast(U32).at[:, pl.ds(pl.multiple_of(which * (L // 2), L // 2), L // 2), :]


def _cols(ref, start, size):
    return jnp.concatenate([_rows(ref, (n,), start, size) for n in range(ref.shape[0])], axis=1)


def _tiled_dot(lhs, w):
    cols, marks = [], []
    for n in range(w.shape[0]):
        for k in range(lhs.shape[1] // 128):
            d = _dot(lhs[:, k * 128:(k + 1) * 128], _rows(w, (n,), k * 128, 128))
            marks.append(d)
            acc = d if k == 0 else acc + d
        cols.append(acc)
    return jnp.concatenate(cols, axis=1), marks


def _put_cols(ref, rows, x):
    for n in range(ref.shape[0]):
        ref[n, rows, :] = x[:, n * 128:(n + 1) * 128]


def _layernorm(x, after=None):
    m = jnp.mean(x, axis=-1, keepdims=True)
    if after is not None:
        m = jnp.concatenate([m + after] * (x.shape[1] // 128), axis=1)
    xc = x - m
    v = jnp.mean(xc * xc, axis=-1, keepdims=True)
    return xc * lax.rsqrt(v + EPS)


def _gelu(x):
    c = 0.7978845608028654
    inner = x * (c + (c * 0.044715) * (x * x))
    hx = 0.5 * x
    return hx + hx * jnp.tanh(inner)


def _unpack(x):
    return pltpu.bitcast(x, BF16)


def _recip(x):
    r = pl.reciprocal(x, approx=True)
    return r * (2.0 - x * r)


def _phi(t):
    return jnp.where(t > 0, t + 1.0, jnp.exp(t))


def _kernel(x_hbm, wq_hbm, wk_hbm, wv_hbm, wo_hbm, beta_hbm, w1_hbm, w2_hbm, w3_hbm, w4_hbm,
            out_hbm,
            xb, xn, xa, ybuf, hbuf, zero, wqkv, wo, w1, w2, w3a, w3, w4,
            qs, pq, kk, pk, vt, zb, ot, mt, gb, beta_ref, x_sems, qkv_sems, w_sems, out_sems):

    def lanes(n):
        return pl.ds(pl.multiple_of(n * 128, 128), 128)

    def x_copy(seg):
        rows = pl.ds(seg * L, L)
        return pltpu.make_async_copy(x_hbm.at[0, rows, :], xb.at[rows, :], x_sems.at[seg + NT - 1])

    def head_copy(p):
        return pltpu.make_async_copy(x_hbm.at[0, lanes(p), :], xb.at[lanes(p), :], x_sems.at[p])

    beta_copy = pltpu.make_async_copy(beta_hbm, beta_ref, w_sems.at[6])

    def out_copy(i):
        rows = pl.ds(pl.multiple_of(i * MB, MB), MB)
        return pltpu.make_async_copy(xb.at[rows, :], out_hbm.at[0, rows, :], out_sems.at[i])

    def qkv_copy(g, i):
        src = (wq_hbm, wk_hbm, wv_hbm)[i]
        return pltpu.make_async_copy(src.at[:, lanes(g)], wqkv.at[g, i], qkv_sems.at[g * 3 + i])

    def w_copy(i, n):
        src, dst = ((wo_hbm, wo), (w1_hbm, w1), (w2_hbm, w2), (w3_hbm, w3a))[i]
        return pltpu.make_async_copy(src.at[:, lanes(n)], dst.at[n], w_sems.at[i])

    wide_copies = [pltpu.make_async_copy(w3_hbm.at[:, pl.ds(W3A, F - W3A)], w3, w_sems.at[4]),
                   pltpu.make_async_copy(w4_hbm, w4, w_sems.at[5])]

    def start_all(copy, i, n=NG):
        for c in range(n):
            copy(i, c).start()

    def wait_all(copy, i, n=NG):
        for c in range(n):
            copy(i, c).wait()

    def launch(k):
        for tok in filter(None, PORD.split('|')[k].split(',')):
            n = int(tok[1])
            (head_copy(n) if tok[0] == 'x' else qkv_copy(n // 3, n % 3)).start()

    launch(0)
    beta_copy.start()

    mt[...] = jnp.zeros(mt.shape, F32)
    zero[0] = 0
    zero_pad = jnp.zeros((NG, PADR, 128), F32)
    hbuf[:, 0:PADR, :] = zero_pad
    hbuf[:, PADR + S:PADR + S + PADR, :] = zero_pad

    def project(slot, n, r, rows, c, memory=True):
        if n == 0:
            qs[slot, rows, :] = (r * QSCALE).astype(BF16)
            pq[slot, rows, :] = _phi(r).astype(BF16)
        elif n == 1:
            kk[slot, rows, :] = r.astype(BF16)
            if not memory:
                return []
            pkf = _phi(r)
            pk[slot, rows, :] = pkf.astype(BF16)
            return [jnp.sum(pkf.reshape(16, 8, 128), axis=0)]
        else:
            vt[slot, c] = r.T.astype(BF16)
        return []

    def qkv_tiles(xslot, g, slot, memory=True):
        xv = _seg(xn, xslot)
        acc, zacc = {}, []

        def tile(c, n, kt):
            d = _dot(_rows(xv, (kt,), c * 128, 128), _rows(wqkv, (g, n), kt * 128, 128))
            acc[0] = d if kt == 0 else acc[0] + d
            if kt < NG - 1:
                return
            zacc.extend(project(slot, n, acc[0], slice(c * 128, (c + 1) * 128), c, memory))
            if n == 1 and c == NT - 1 and memory:
                zb[slot] = jnp.sum(sum(zacc), axis=0, keepdims=True)

        return [(128, partial(tile, c, n, kt))
                for c in range(NT) for n in ((0, 1, 2) if c < NT - 1 else (2, 1, 0)) for kt in range(NG)]

    class Group:
        def __init__(self, g, slot):
            self.g, self.slot = g, slot
            self.mem, self.rden, self.parts, self.upd = {}, {}, {}, {}
            self.diag, self.outs = {}, {}

        def retrieve(self, j):
            mem = _dot_nt(mt[self.g].astype(BF16), _rows(pq, (self.slot,), j * 128, 128))
            self.mem[j] = mem
            self.rden[j] = _recip(mem[128:136] + 1e-6)

        def update(self, t, lo, n):
            g, slot = self.g, self.slot
            d = _dot(_rows(vt, (slot, t), lo, n), _rows(pk, (slot,), t * 128, 128))
            for r in range(lo, lo + n, DH):
                part = d[r - lo:r - lo + DH]
                self.upd[r] = part if t == 0 else self.upd[r] + part
            if t < NT - 1 or lo + n < 128:
                return
            upd = jnp.concatenate([self.upd[r] for r in range(0, 128, DH)], axis=0)
            row = lax.broadcasted_iota(jnp.int32, (128, 128), 0)
            col = lax.broadcasted_iota(jnp.int32, (128, 128), 1)
            mt[g, 0:128, :] = mt[g, 0:128, :] + jnp.where(row // DH == col // DH, upd, 0.0)
            zrow = lax.broadcasted_iota(jnp.int32, (MROWS - 128, 128), 0)
            zlane = lax.broadcasted_iota(jnp.int32, (MROWS - 128, 128), 1)
            mt[g, 128:MROWS, :] = mt[g, 128:MROWS, :] + jnp.where(zrow == zlane // DH, zb[slot], 0.0)

        def masked_q(self, lo, n, h):
            lane = lax.broadcasted_iota(jnp.int32, (n, 128), 1)
            q = qs.bitcast(U32)[self.slot, lo:lo + n, :]
            return jnp.where((lane >= h * DH) & (lane < (h + 1) * DH), q, jnp.uint32(0))

        def scores(self, j, h):
            self.parts[j, h] = []
            return _dot_nt(_rows(kk, (self.slot,), 0, j * 128 + 32), _unpack(self.masked_q(j * 64, 64, h)))

        def outer(self, j, ha, hb):
            lane = lax.broadcasted_iota(jnp.int32, (16, 128), 1)
            kp = kk.bitcast(U32)
            keys = jnp.where((lane // DH) % 2 == hb % 2, kp[self.slot, j * 64 + 48:j * 64 + 64, :],
                             kp[self.slot, j * 64 + 16:j * 64 + 32, :])
            qc = jnp.concatenate([self.masked_q(j * 64 + 48, 16, hb), self.masked_q(j * 64 + 16, 48, ha)], axis=0)
            st = _dot_nt(_unpack(keys), _unpack(qc))
            self.diag[j, ha, 0] = st
            self.diag[j, hb, 2] = pltpu.roll(st, 96, 1)

        def inner(self, j, h):
            qc = jnp.concatenate([self.masked_q(j * 64 + 32, 32, h + d) for d in range(2)], axis=0)
            st = _dot_nt(_rows(kk, (self.slot,), j * 128 + 64, 32), _unpack(qc))
            self.diag[j, h, 1] = pltpu.roll(st, 64, 1)
            self.diag[j, h + 1, 1] = st

        def weigh(self, j, h, t, st):
            if t == j:
                st = jnp.concatenate([st[t * 128:t * 128 + 32]] + [self.diag[j, h, i] for i in range(3)], axis=0)
                key_i = lax.broadcasted_iota(jnp.int32, (128, 128), 0)
                qry_i = lax.broadcasted_iota(jnp.int32, (128, 128), 1)
                st = jnp.where(key_i <= qry_i, st, NEG)
            else:
                st = st[t * 128:(t + 1) * 128]
            m = jnp.max(st, axis=0, keepdims=True)
            p = jnp.exp2(st - m)
            l = jnp.sum(p.reshape(16, 8, 128), axis=0)
            pv = _dot(_rows(vt, (self.slot, t), h * DH, DH), p.astype(BF16))
            parts = self.parts[j, h]
            parts.append((m, l, pv))
            if len(parts) < j + 1:
                return
            gate = gb[pl.ds(self.g * HPG + h, 1), :]
            o = self.mem[j][h * DH:(h + 1) * DH] * (gate * self.rden[j][h:h + 1])
            if j == 0:
                o = o + pv * ((1.0 - gate) * _recip(jnp.sum(l, axis=0, keepdims=True)))
            else:
                mx = reduce(jnp.maximum, [pt[0] for pt in parts])
                alphas = [jnp.exp2(pt[0] - mx) for pt in parts]
                lp = sum(al * pt[1] for al, pt in zip(alphas, parts))
                r2 = (1.0 - gate) * _recip(jnp.sum(lp, axis=0, keepdims=True))
                for al, pt in zip(alphas, parts):
                    o = o + pt[2] * (al * r2)
            outs = self.outs.setdefault(j, {})
            outs[h] = o
            if len(outs) == HPG:
                o4 = jnp.concatenate([outs[i] for i in range(HPG)], axis=0)
                ot[self.g, j * 128:(j + 1) * 128, :] = o4.T.astype(BF16)

    def attn_block(groups, fillers, final=False):
        free = [0] * 4
        rate = RATEF if final else RATE
        lead, start = [], 0
        for grp in groups:
            for j in range(NT):
                lead.append((start, MROWS, partial(grp.retrieve, j), None))
                for h in range(HPG):
                    dur = 128 * j + 32
                    lead.append((start, dur, partial(grp.scores, j, h), (grp, j, h, dur)))
                    if h % 2 == 0:
                        for q, fn in enumerate((partial(grp.outer, j, h + 1, h), partial(grp.inner, j, h),
                                                partial(grp.outer, j, h, h + 1))):
                            lead.append((start + max(CMIN, dur - CLEAD) + q * CGAP, PVD, fn, (grp, j, h, None)))
                    start += int((128 * j + SB) * rate * 4400 / (3072 + 16 * SB))
                    if j == NT - 1 and not final:
                        n = 128 if grp is not groups[-1] else UROWS[h]
                        for lo in range(0, 128, n):
                            lead.append((start - 256 if grp is not groups[-1] else 10 ** 6, n,
                                         partial(grp.update, h, lo, n), None))
        lead.sort(key=lambda e: e[0])
        ready, diag = [], {}
        fillers = list(fillers)
        total = len(fillers)

        def fed(fn):
            if not final or fn.func.__self__ is not groups[-1]:
                return True
            return total - len(fillers) >= min(total, 3 * NG * (fn.args[0] + 1) + GSL)

        def issue(dur):
            i = min(range(4), key=lambda m: free[m])
            t0 = free[i]
            free[i] = t0 + dur
            return t0

        for _ in range(NF):
            dur, fn = fillers.pop(0)
            issue(dur)
            fn()
        while lead or ready or fillers:
            now = min(free)
            if ready and (ready[0][0] <= now or not (lead or fillers)):
                issue(PVD)
                ready.pop(0)[1]()
            elif final and not fillers and lead[0][0] > now:
                free[free.index(now)] = min([lead[0][0]] + [e[0] for e in ready[:1]])
            elif lead and (lead[0][0] <= now or not fillers) and fed(lead[0][2]):
                _, dur, fn, qk = lead.pop(0)
                t0 = issue(dur)
                res = fn()
                if qk is not None:
                    grp, j, h, full = qk
                    if full:
                        ready += [(t0 + 128 * (t + 1) + DELAY, partial(grp.weigh, j, h, t, res)) for t in range(j)]
                    for hd in (h,) if full else (h, h + 1):
                        need = diag.setdefault((grp.slot, j, hd), [])
                        need.append((t0 + dur + (0 if full else DD), res))
                        if len(need) == 4:
                            ready.append((max(e[0] for e in need) + DELAY,
                                          partial(grp.weigh, j, hd, j, [e[1] for e in need if e[1] is not None][0])))
                    ready.sort(key=lambda e: e[0])
            else:
                dur, fn = fillers.pop(0)
                issue(dur)
                fn()

    def norm_input(src, dst, lo, n, after=None):
        x = src[lo:lo + n, :].astype(F32)
        _put_cols(dst, slice(lo, lo + n), _layernorm(x, after).astype(BF16))

    def blank(v):
        return jnp.where(zero[0] != 0, v, 0.0)

    def norm_tile(lo, n):
        rows = pl.ds(pl.multiple_of(lo, n), n)
        norm_input(xb.at[rows, :], xn.at[:, rows, :], 0, n)

    head_copy(0).wait()
    launch(1)
    norm_input(xb, xn, 0, 128)
    beta_copy.wait()
    beta = beta_ref[...].astype(F32)
    g_row = 1.0 / (1.0 + jnp.exp(-beta))
    eye = lax.broadcasted_iota(jnp.int32, (H, H), 0) == lax.broadcasted_iota(jnp.int32, (H, H), 1)
    g_col = jnp.sum(jnp.where(eye, g_row, 0.0), axis=1, keepdims=True)
    gb[...] = jnp.broadcast_to(g_col, (H, 128))

    def first(p, z, arrive=None):
        lhs = xn.bitcast(U32).at[:, pl.ds(pl.multiple_of(p * 64, 64), 64), :]
        for n in range(3):
            if arrive:
                arrive(n)
            r, _ = _tiled_dot(_cols(lhs, 0, 128), wqkv.bitcast(U32).at[0, pl.ds(n, 1)])
            z = sum(project(0, n, r, lanes(p), p), z)
        return z

    def weights(n):
        qkv_copy(0, n).wait()
        launch(2 + n)
        if n == XP:
            head_copy(1).wait()
            launch(5)
            norm_input(xb, xn, 128, 128)

    def rest(p, z):
        for q in range(1, NT - 1):
            @pl.when(p == q)
            def _():
                head_copy(q + 1).wait()
                launch(5 + q)
        z = first(p, z)
        norm_tile(jnp.minimum(p + 1, NT - 1) * 128, 128)
        return z
    z0 = first(0, jnp.zeros((8, 128), F32), weights)
    zb[0] = jnp.sum(lax.fori_loop(1, NT, rest, z0), axis=0, keepdims=True)

    def phase_a(t):
        s = t % NSEG
        r0 = pl.multiple_of(s * L, L)
        xslot = t % 2

        @pl.when(t == NSEG)
        def _():
            mt[...] = jnp.zeros(mt.shape, F32)

        def body(i, c):
            g = 2 * i

            @pl.when(t == 0)
            def _():
                for j in range(3):
                    qkv_copy(g + 1, j).wait()

                @pl.when(i < NG // 2 - 1)
                def _():
                    for j in range(3):
                        qkv_copy(g + 2, j).wait()

                @pl.when(i == 0)
                def _():
                    for g2 in range(3, NG):
                        for j in range(3):
                            qkv_copy(g2, j).start()
                    x_copy(1).start()

                @pl.when(i == 1)
                def _():
                    start_all(w_copy, 0)
                    start_all(w_copy, 1)
                    x_copy(2).start()
                    x_copy(3).start()

                @pl.when(i == NG // 2 - 1)
                def _():
                    x_copy(1).wait()
                    _each(L // XL, lambda p: norm_tile(L + p * XL, XL))

            last = i == NG // 2 - 1
            fa = qkv_tiles(xslot, g + 1, 1)
            fb = qkv_tiles(jnp.where(last, 1 - xslot, xslot), jnp.where(last, 0, g + 2), 0)
            attn_block([Group(g, 0), Group(g + 1, 1)], fa + fb)
            return c
        lax.fori_loop(0, jnp.where(t == NSTEP - 1, NG // 2 - 1, NG // 2), body, 0)

        @pl.when(t == NSTEP - 1)
        def _():
            attn_block([Group(NG - 2, 0), Group(NG - 1, 1)], qkv_tiles((NSTEP - 1) % 2, NG - 1, 1, False), True)

        @pl.when(t == 0)
        def _():
            wait_all(w_copy, 0)
            wait_all(w_copy, 1)
            x_copy(2).wait()
            x_copy(3).wait()
            start_all(w_copy, 2)
            start_all(w_copy, 3, W3A // 128)
            for cp in wide_copies:
                cp.start()

        sub = L // SUBA
        hview = hbuf.at[:, pl.ds(r0, L + 2 * PADR), :]
        xav, yv = (r.at[pl.ds(r0, L), :] for r in (xa, ybuf))
        xv, xnext = (xb.at[pl.ds(pl.multiple_of(q * L, L), L), :] for q in (s, (t + 2) % NSEG))
        xnv = xn.at[:, pl.ds(pl.multiple_of(xslot * L, L), L), :]
        ys, x2s, res, pend = {}, {}, {}, []

        def tile_of(dep, k):
            return blank(res[dep][k][0:LNC]) if k >= 0 else None

        def op(i, dep):
            attn, res['o%d' % i] = _tiled_dot(_cols(ot, i * sub, sub), wo)
            x2s[i] = xv[i * sub:(i + 1) * sub, :].astype(F32) + attn
            xav[i * sub:(i + 1) * sub, :] = x2s[i]

        def ln(i, dep):
            zs = []
            for c in range(sub // LNC):
                after = tile_of(dep, (c * LNC * LUSE) // sub - 1)
                if pend and c == ANC:
                    pend.clear()
                    mark = xn.bitcast(U32)[0, pl.ds(pl.multiple_of(zero[0], 8), LNC), :]
                    mark = blank(pltpu.bitcast(mark, F32))
                    after = mark if after is None else after + mark
                y = _layernorm(x2s[i][c * LNC:(c + 1) * LNC], after)
                yv[i * sub + c * LNC:i * sub + (c + 1) * LNC, :] = y
                zs.append(_layernorm(y).astype(BF16))
            ys[i] = jnp.concatenate(zs, axis=0)

        def up(i, dep):
            pre, res['u%d' % i] = _tiled_dot(ys[i], w1)
            _put_cols(hview, slice(PADR + i * sub, PADR + (i + 1) * sub), _gelu(pre))

        toks = AORD.split(',')

        def nrm(i, dep):
            same = [tk for tk in toks if tk[0] == 'n' and tk[2:] == dep]
            pos = same.index('n%d%s' % (i, dep))
            pend.append(i)
            for c in range(0, sub, LNC):
                norm_input(xnext, xnv, i * sub + c, LNC,
                           tile_of(dep, ((pos * sub + c) * NUSE) // (len(same) * sub) - 1))

        for tok in toks:
            {'o': op, 'u': up, 'n': nrm, 'l': ln}[tok[0]](int(tok[1]), tok[2:])

    def phase_b(t, i):
        tile = (t % NSEG) * (L // MB) + i
        r0 = pl.multiple_of(tile * MB, MB)
        hview = hbuf.at[:, pl.ds(r0, MB + 2 * PADR), :]
        shifts = (-1, -1, 1, 1, -2, -2, 2, 2)
        sub = MB // SUBB
        x1s, ts, xn2, has = [], [], [], []

        def norm(x1, marks, use):
            zs = []
            for c in range(0, sub, LNC):
                k = (c * use) // sub - 1
                zs.append(_layernorm(x1[c:c + LNC], blank(marks[k][0:LNC]) if k >= 0 else None).astype(BF16))
            xn2.append(jnp.concatenate(zs, axis=0))

        for j in range(SUBB):
            rows = pl.ds(r0 + j * sub, sub)
            lo = PADR + j * sub
            hs_in = jnp.concatenate(
                [hview[g, lo + shifts[g]:lo + shifts[g] + sub, :].astype(BF16) for g in range(NG)], axis=1)
            hs, marks = _tiled_dot(hs_in, w2)
            x1s.append(ybuf[rows, :] + hs)
            ts.append(xa[rows, :] + x1s[j])
        norm(x1s[0], marks, BU0)
        pre, marks = _tiled_dot(xn2[0], w3a)
        has.append(_gelu(pre).astype(BF16))
        norm(x1s[1], marks, BU1)
        has.append(_gelu(_tiled_dot(xn2[1], w3a)[0]).astype(BF16))
        ha = jnp.concatenate(has, axis=0)
        hb = _gelu(_dot(jnp.concatenate(xn2, axis=0), w3[...])).astype(BF16)
        h2 = jnp.concatenate([ha, hb], axis=1)
        res = jnp.concatenate(ts, axis=0) + _dot(h2, w4[...])
        xb[pl.ds(r0, MB), :] = res.astype(BF16)

        @pl.when(t >= NSTEP - NSEG)
        def _():
            out_copy(tile).start()

    def step(t, c):
        @pl.when(t < NSTEP)
        def _():
            phase_a(t)

        @pl.when(t == 1)
        def _():
            wait_all(w_copy, 2)
            wait_all(w_copy, 3, W3A // 128)
            for cp in wide_copies:
                cp.wait()

        @pl.when(t > 0)
        def _():
            _each(L // MB, lambda i: phase_b(t - 1, i))
        return c
    lax.fori_loop(0, NSTEP + 1, step, 0)

    for i in range(S // MB):
        out_copy(i).wait()


@jax.jit
def pallas_interleave_layers__memory_aug_infini_attn__mixer_s_mlp__prompt_kernel(
    A_x: jax.Array,
    A_wq: jax.Array,
    A_wk: jax.Array,
    A_wv: jax.Array,
    A_wo: jax.Array,
    A_beta: jax.Array,
    B_x: jax.Array,
    B_w1: jax.Array,
    B_w2: jax.Array,
    B_w3: jax.Array,
    B_w4: jax.Array,
):
    del B_x
    hbm = pl.BlockSpec(memory_space=pl.ANY)
    scratch = [
        pltpu.VMEM((S, D), BF16),
        pltpu.VMEM((NG, 2 * L, 128), BF16),
        pltpu.VMEM((S, D), F32),
        pltpu.VMEM((S, D), F32),
        pltpu.VMEM((NG, S + 2 * PADR, 128), F32),
        pltpu.SMEM((1,), jnp.int32),
        pltpu.VMEM((NG, 3, D, 128), BF16),
        pltpu.VMEM((NG, D, 128), BF16),
        pltpu.VMEM((NG, D, 128), BF16),
        pltpu.VMEM((NG, D, 128), BF16),
        pltpu.VMEM((W3A // 128, D, 128), BF16),
        pltpu.VMEM((D, F - W3A), BF16),
        pltpu.VMEM((F, D), BF16),
        pltpu.VMEM((2, L, 128), BF16),
        pltpu.VMEM((2, L, 128), BF16),
        pltpu.VMEM((2, L, 128), BF16),
        pltpu.VMEM((2, L, 128), BF16),
        pltpu.VMEM((2, NT, 128, 128), BF16),
        pltpu.VMEM((2, 1, 128), F32),
        pltpu.VMEM((NG, L, 128), BF16),
        pltpu.VMEM((NG, MROWS, 128), F32),
        pltpu.VMEM((H, 128), F32),
        pltpu.VMEM((1, H), BF16),
        pltpu.SemaphoreType.DMA((NSEG + NT - 1,)),
        pltpu.SemaphoreType.DMA((3 * NG,)),
        pltpu.SemaphoreType.DMA((7,)),
        pltpu.SemaphoreType.DMA((S // MB,)),
    ]
    return pl.pallas_call(
        _kernel,
        out_shape=jax.ShapeDtypeStruct(A_x.shape, A_x.dtype),
        in_specs=[hbm] * 10,
        out_specs=hbm,
        scratch_shapes=scratch,
        compiler_params=pltpu.CompilerParams(vmem_limit_bytes=120 * 1024 * 1024),
    )(A_x, A_wq, A_wk, A_wv, A_wo, A_beta.reshape(1, H), B_w1, B_w2, B_w3, B_w4)
```
